```python
import jax
import jax.numpy as jnp

def _softmax(x, axis=-1):
    return jax.nn.softmax(x, axis=axis)

def _gelu(x):
    return jax.nn.gelu(x, approximate=True)

def _silu(x):
    return jax.nn.silu(x)

def _sigmoid(x):
    return jax.nn.sigmoid(x)

def _layernorm(x, axis=-1, eps=1e-05):
    m = jnp.mean(x, axis=axis, keepdims=True)
    v = jnp.var(x, axis=axis, keepdims=True)
    return (x - m) / jnp.sqrt(v + eps)

def _scatter_add(tgt, idx, src, axis=0):
    return tgt.at[idx].add(src)

def _segment_sum(src, seg, n):
    return jax.ops.segment_sum(src, seg, n)

class _Rng:

    def __init__(self, key):
        self._k = key

    def _next(self):
        self._k, sub = jax.random.split(self._k)
        return sub

    def normal(self, shape):
        return jax.random.normal(self._next(), shape, dtype=jnp.bfloat16)

    def randint(self, lo, hi, shape):
        return jax.random.randint(self._next(), shape, lo, hi, dtype=jnp.int32)

    def uniform(self, shape, lo=0.0, hi=1.0):
        return jax.random.uniform(self._next(), shape, jnp.bfloat16, lo, hi)

    def permutation(self, n):
        return jax.random.permutation(self._next(), n)
kernel_name = 'adaLN_cond__ssm_conv_h3__glu_gated_reglu__prompt'

def setup_inputs():
    _rng = _Rng(jax.random.key(int.from_bytes(__import__("os").urandom(4), "little")))
    _w = lambda a: (lambda t: t.astype(jnp.bfloat16) if jnp.issubdtype(t.dtype, jnp.floating) else t)(jnp.asarray(a))

    def _A_setup():
        B, S, D = (1, 2048, 640)
        ks = 4
        return {'q': _w((lambda *s: _rng.normal(s) * 0.05)(B, S, D)), 'k': _w((lambda *s: _rng.normal(s) * 0.05)(B, S, D)), 'v': _w((lambda *s: _rng.normal(s) * 0.05)(B, S, D)), 'shift_k': _w((lambda *s: _rng.normal(s) * 0.05)(D, ks) * 0.5), 'ssm_k': _w((lambda *s: _rng.normal(s) * 0.05)(D, S) * (1.0 / S ** 0.5)), 'ssm_D': _w((lambda *s: _rng.normal(s) * 0.05)(D))}
    _A_in = _A_setup()

    def _B_setup():
        B, S, D, F = (1, 2048, 640, 1536)
        return {'x': _w((lambda *s: _rng.normal(s) * 0.05)(B, S, D)), 'W_gate': _w((lambda *s: _rng.normal(s) * 0.05)(D, F) * (2.0 / D) ** 0.5), 'W_up': _w((lambda *s: _rng.normal(s) * 0.05)(D, F) * (2.0 / D) ** 0.5), 'W_down': _w((lambda *s: _rng.normal(s) * 0.05)(F, D) * (1.0 / F) ** 0.5)}
    _B_in = _B_setup()
    return {'A_q': _A_in['q'], 'A_k': _A_in['k'], 'A_v': _A_in['v'], 'A_shift_k': _A_in['shift_k'], 'A_ssm_k': _A_in['ssm_k'], 'A_ssm_D': _A_in['ssm_D'], 'B_x': _B_in['x'], 'B_W_gate': _B_in['W_gate'], 'B_W_up': _B_in['W_up'], 'B_W_down': _B_in['W_down'], 'c': _w((lambda *s: _rng.normal(s) * 0.05)(1, 640)), 'w_mod': _w((lambda *s: _rng.normal(s) * 0.05)(640, 6 * 640) * 640 ** (-0.5))}

def reference(A_q, A_k, A_v, A_shift_k, A_ssm_k, A_ssm_D, B_x, B_W_gate, B_W_up, B_W_down, c, w_mod):

    def _A_ref(q, k, v, shift_k, ssm_k, ssm_D):
        B, S, D = q.shape
        ks = shift_k.shape[-1]
        k_pad = jnp.pad(k, ((0, 0), (ks - 1, 0), (0, 0)))
        k_shift = jnp.zeros_like(k)
        for t in range(ks):
            k_shift = k_shift + k_pad[:, t:t + S, :] * shift_k[:, ks - 1 - t][None, None, :]
        kv = k_shift * v
        L = 2 * S
        kv_pad = jnp.pad(kv, ((0, 0), (0, S), (0, 0)))
        kf_pad = jnp.pad(ssm_k, ((0, 0), (0, S)))
        kv_f = (lambda x, axes=(-2, -1): jnp.fft.rfft2(x.astype(jnp.float32), axes=axes))(kv_pad[:, None, :, :], axes=(1, 2))
        kf_f = (lambda x, axes=(-2, -1): jnp.fft.rfft2(x.astype(jnp.float32), axes=axes))(kf_pad[:, None, :], axes=(1, 2))
        kf_f = (lambda x, *d: x.transpose(*d))(kf_f, 1, 2, 0)
        y_f = kv_f * kf_f[None, :, :, :]
        y = (lambda x, s, axes=(-2, -1): jnp.fft.irfft2(x, s=s, axes=axes).astype(jnp.bfloat16))(y_f, (1, L), axes=(1, 2))[:, 0, :S, :]
        y = y + kv * ssm_D[None, None, :]
        return q * y

    def _B_ref(x, W_gate, W_up, W_down):
        gate = jnp.einsum('bsd,df->bsf', x, W_gate)
        up = jnp.einsum('bsd,df->bsf', x, W_up)
        gate = gate * (lambda x, dt: x.astype(dt))(gate > 0, gate.dtype)
        h = gate * up
        return jnp.einsum('bsf,fd->bsd', h, W_down)
    x = A_q
    mod = (_silu(c) @ w_mod).reshape(c.shape[0], 6, 1, -1)
    sa, ca, ga, sb, cb, gb = (mod[:, 0].copy(), mod[:, 1].copy(), mod[:, 2].copy(), mod[:, 3].copy(), mod[:, 4].copy(), mod[:, 5].copy())
    h = _layernorm(x, axis=-1) * (1 + ca) + sa
    x = x + ga * _A_ref(h, A_k, A_v, A_shift_k, A_ssm_k, A_ssm_D)
    h = _layernorm(x, axis=-1) * (1 + cb) + sb
    x = x + gb * _B_ref(h, B_W_gate, B_W_up, B_W_down)
    return x
```

```python
import functools
import math

import jax
import jax.numpy as jnp
import numpy as np
from jax import lax
import jax.experimental.pallas as pl
import jax.experimental.pallas.tpu as pltpu

C = 128
LANES = 128
EPS = 1e-5


def _kernel(q_hbm, k_hbm, v_hbm, shift_hbm, ssmk_hbm, ssmd_hbm, wg_hbm, wu_hbm, wd_hbm,
            c_hbm, wmod_hbm, o_hbm,
            q_s, k_s, v_s, ssmk_s, wg_s, wu_s, wd_s, wmod_s, shift_s, ssmd_s, c_s,
            kf_s, kp_s, kraw_s, u_s, yb_s, y_s, x1_s, h2_s, h_s, out_s, sems,
            *, S, D, F, cfg):
    f32, bf16 = jnp.float32, jnp.bfloat16
    NT = D // LANES
    NA = S // C
    TS = 2 * C
    NS = S // TS
    TN = cfg.get("tn", 128)
    NF = F // TN

    sem_count = [0]
    dmas = {}

    def mk(name, src, dst):
        i = sem_count[0]
        sem_count[0] += 1
        dmas[name] = pltpu.make_async_copy(src, dst, sems.at[i])

    mk("c", c_hbm, c_s)
    mk("shift", shift_hbm, shift_s)
    mk("ssmd", ssmd_hbm, ssmd_s)
    for t in range(NS):
        r = pl.ds(t * TS, TS)
        mk(("ssmk", t), ssmk_hbm.at[:, r], ssmk_s.at[:, r])
        mk(("k", t), k_hbm.at[r, :], k_s.at[r, :])
        mk(("v", t), v_hbm.at[r, :], v_s.at[r, :])
        mk(("q", t), q_hbm.at[r, :], q_s.at[r, :])
    for j in range(6):
        cs = pl.ds(j * D, D)
        mk(("wmod", j), wmod_hbm.at[:, cs], wmod_s.at[:, cs])
    WG = cfg.get("wg_dma", 256)
    for j in range(F // WG):
        cs = pl.ds(j * WG, WG)
        mk(("wg", j), wg_hbm.at[:, cs], wg_s.at[:, cs])
        mk(("wu", j), wu_hbm.at[:, cs], wu_s.at[:, cs])
    for j in range(NT):
        cs = pl.ds(j * LANES, LANES)
        mk(("wd", j), wd_hbm.at[:, cs], wd_s.at[:, cs])
    for t in range(NS):
        r = pl.ds(t * TS, TS)
        mk(("out", t), out_s.at[r, :], o_hbm.at[r, :])

    order = ["c", "shift", "ssmd"]
    for t in range(NS):
        order += [("ssmk", t), ("k", t), ("v", t)]
    order += [("wmod", 0), ("wmod", 1), ("q", 0), ("wmod", 2), ("wmod", 3), ("wmod", 4)]
    for j in range(F // WG):
        order += [("wg", j), ("wu", j)]
    order += [("q", 1)]
    order += [("wd", j) for j in range(NT)]
    order += [("wmod", 5)] + [("q", t) for t in range(2, NS)]
    for name in order:
        dmas[name].start()
    waited = set()

    def wait(*names):
        for n in names:
            if n not in waited:
                waited.add(n)
                dmas[n].wait()

    def table(shape, fdim, ndim, f_off):
        f = lax.broadcasted_iota(jnp.int32, shape, fdim)
        n = lax.broadcasted_iota(jnp.int32, shape, ndim)
        m = ((4 * f + 1) * n + f_off) & (4 * C - 1)
        return jnp.sin(m.astype(f32) * (2.0 * math.pi / (4 * C)))

    Fm = jnp.concatenate([table((C, C), 0, 1, C), table((C, C), 0, 1, 0)], axis=0).astype(bf16)
    Gm = (jnp.concatenate([table((C, C), 1, 0, C), table((C, C), 1, 0, 0)], axis=1)
          * (1.0 / C)).astype(bf16)

    wait("c", "shift", "ssmd")
    sel = (lax.broadcasted_iota(jnp.int32, (16, LANES), 0)
           == lax.broadcasted_iota(jnp.int32, (16, LANES), 1)).astype(bf16)
    shift_rows = lax.dot_general(sel, shift_s[...], (((1,), (1,)), ((), ())),
                                 preferred_element_type=f32)
    wtap = [shift_rows[j:j + 1, :] for j in range(4)]
    ssmd = ssmd_s[...].astype(f32)

    def kvprep(t):
        r0 = t * TS
        outs = []
        for jt in range(NT):
            ls = slice(jt * LANES, (jt + 1) * LANES)
            kk = k_s[r0:r0 + TS, ls].astype(f32)
            if t == 0:
                kf_s[jt, 0:8, :] = jnp.zeros((8, LANES), f32)
            else:
                kf_s[jt, 0:8, :] = k_s[r0 - 16:r0, ls].astype(f32)[8:16]
            kf_s[jt, 8:8 + TS, :] = kk
            acc = kk * wtap[0][:, ls]
            for j in range(1, 4):
                acc = acc + kf_s[jt, 8 - j:8 - j + TS, :] * wtap[j][:, ls]
            outs.append((acc * v_s[r0:r0 + TS, ls].astype(f32)).astype(bf16))
        return jnp.concatenate(outs, axis=1)

    def dft_k(a):
        kc = ssmk_s[:, a * C:(a + 1) * C]
        kk = lax.dot_general(Fm, kc, (((1,), (1,)), ((), ())), preferred_element_type=f32)
        kr, ki = kk[0:C], kk[C:2 * C]
        if a == 0:
            kr = kr + ssmd
            kp_s[0, 0] = kr
            kp_s[0, 1] = ki
        else:
            kp_s[a, 0] = kr + kraw_s[(a - 1) % 2, 1]
            kp_s[a, 1] = ki - kraw_s[(a - 1) % 2, 0]
        kraw_s[a % 2, 0] = kr
        kraw_s[a % 2, 1] = ki
        return kk

    def dft_u(t, kv):
        res = []
        for o in range(2):
            uu = jnp.dot(Fm, kv[o * C:(o + 1) * C], preferred_element_type=f32)
            u_s[2 * t + o, 0] = uu[0:C]
            u_s[2 * t + o, 1] = uu[C:2 * C]
            res.append(uu)
        return res

    def x_unit(t, jt, r, anchor=None):
        a0 = 2 * t
        ls = slice(jt * LANES, (jt + 1) * LANES)
        res = []
        for hh in range(2):
            rs = slice(r * 16 + hh * 8, r * 16 + hh * 8 + 8)
            acc = [[None, None], [None, None]]
            us = None
            for m in range(a0 + 2):
                kr = kp_s[m, 0, rs, ls]
                ki = kp_s[m, 1, rs, ls]
                if anchor is not None:
                    an = anchor(hh, m)
                    if an is not None:
                        kr = jnp.where(never, an, kr)
                if m == 0:
                    us = [(u_s[a0, 0, rs, ls], u_s[a0, 1, rs, ls]),
                          (u_s[a0 + 1, 0, rs, ls], u_s[a0 + 1, 1, rs, ls])]
                else:
                    new = (u_s[a0 - m, 0, rs, ls], u_s[a0 - m, 1, rs, ls]) if a0 - m >= 0 else None
                    us = [new, us[0]]
                for o in range(2):
                    if us[o] is None:
                        continue
                    ur, ui = us[o]
                    pr = kr * ur - ki * ui
                    pi = kr * ui + ki * ur
                    acc[o][0] = pr if acc[o][0] is None else acc[o][0] + pr
                    acc[o][1] = pi if acc[o][1] is None else acc[o][1] + pi
            res.append(acc)
        for o in range(2):
            for p in range(2):
                yb_s[t % 2, o, p * C + r * 16:p * C + (r + 1) * 16, ls] = (
                    jnp.concatenate([res[0][o][p], res[1][o][p]], axis=0).astype(bf16))

    def x_stage(t):
        for jt in range(NT):
            for r in range(C // 16):
                x_unit(t, jt, r)

    def inv(t):
        for o in range(2):
            y_s[t, o * C:(o + 1) * C, :] = jnp.dot(Gm, yb_s[t % 2, o], preferred_element_type=f32)

    def modvec(j, sc):
        wait(("wmod", j))
        m = jnp.dot(sc, wmod_s[:, j * D:(j + 1) * D], preferred_element_type=f32)
        return m[0:1, :]

    def layernorm(x):
        mu = jnp.mean(x, axis=1, keepdims=True)
        xc = x - mu
        var = jnp.mean(xc * xc, axis=1, keepdims=True)
        return xc * lax.rsqrt(var + EPS)

    def e1(t, mod):
        sa, ca, ga, sb, cb = mod
        RG = 16
        for g in range(TS // RG):
            rows = slice(t * TS + g * RG, t * TS + (g + 1) * RG)
            lr = slice(g * RG, (g + 1) * RG)
            x = q_s[rows, :].astype(f32)
            h = layernorm(x) * ca + sa
            x1 = x + ga * (h * y_s[t, lr, :])
            x1_s[t % 2, lr, :] = x1
            h2_s[lr, :] = (layernorm(x1) * cb + sb).astype(bf16)

    def glu(t, gb):
        for j in range(NF):
            cs = slice(j * TN, (j + 1) * TN)
            for w in range(j * TN // WG, ((j + 1) * TN + WG - 1) // WG):
                wait(("wg", w), ("wu", w))
            g = jnp.dot(h2_s[...], wg_s[:, cs], preferred_element_type=f32)
            u = jnp.dot(h2_s[...], wu_s[:, cs], preferred_element_type=f32)
            h_s[:, cs] = (jnp.maximum(g, 0.0) * u).astype(bf16)
        for j in range(NT):
            cs = slice(j * LANES, (j + 1) * LANES)
            wait(("wd", j))
            d = jnp.dot(h_s[...], wd_s[:, cs], preferred_element_type=f32)
            out_s[t * TS:(t + 1) * TS, cs] = (x1_s[t % 2, :, cs] + gb()[:, cs] * d).astype(bf16)
        dmas[("out", t)].start()

    never = None
    cc = c_s[...].astype(f32)
    sc = (cc * jax.nn.sigmoid(cc)).astype(bf16)
    sc = jnp.broadcast_to(sc, (16, D))

    for t in range(NS):
        wait(("ssmk", t))
        dft_k(2 * t)
        dft_k(2 * t + 1)
        wait(("k", t), ("v", t))
        kv = kvprep(t)
        dft_u(t, kv)
        if t >= 1:
            x_stage(t - 1)
        if t >= 2:
            inv(t - 2)
    x_stage(NS - 1)
    inv(NS - 2)
    mod = [modvec(j, sc) for j in range(5)]
    mod[1] = mod[1] + 1.0
    mod[4] = mod[4] + 1.0
    inv(NS - 1)
    gbv = []

    def gb():
        if not gbv:
            gbv.append(modvec(5, sc))
        return gbv[0]

    for t in range(NS):
        wait(("q", t))
        e1(t, mod)
        glu(t, gb)
    for t in range(NS):
        dmas[("out", t)].wait()


def _build(S, D, F, cfg):
    f32, bf16 = jnp.float32, jnp.bfloat16
    NT, NA, TS, NS = D // LANES, S // C, 2 * C, S // (2 * C)
    scratch = [
        pltpu.VMEM((S, D), bf16),
        pltpu.VMEM((S, D), bf16),
        pltpu.VMEM((S, D), bf16),
        pltpu.VMEM((D, S), bf16),
        pltpu.VMEM((D, F), bf16),
        pltpu.VMEM((D, F), bf16),
        pltpu.VMEM((F, D), bf16),
        pltpu.VMEM((D, 6 * D), bf16),
        pltpu.VMEM((D, LANES), bf16),
        pltpu.VMEM((1, D), bf16),
        pltpu.VMEM((1, D), bf16),
        pltpu.VMEM((NT, 8 + TS, LANES), f32),
        pltpu.VMEM((NA, 2, C, D), f32),
        pltpu.VMEM((2, 2, C, D), f32),
        pltpu.VMEM((NA, 2, C, D), f32),
        pltpu.VMEM((2, 2, 2 * C, D), bf16),
        pltpu.VMEM((NS, TS, D), f32),
        pltpu.VMEM((2, TS, D), f32),
        pltpu.VMEM((TS, D), bf16),
        pltpu.VMEM((TS, F), bf16),
        pltpu.VMEM((S, D), bf16),
        pltpu.SemaphoreType.DMA((96,)),
    ]
    return pl.pallas_call(
        functools.partial(_kernel, S=S, D=D, F=F, cfg=cfg),
        in_specs=[pl.BlockSpec(memory_space=pl.ANY)] * 11,
        out_specs=pl.BlockSpec(memory_space=pl.ANY),
        out_shape=jax.ShapeDtypeStruct((S, D), bf16),
        scratch_shapes=scratch,
        compiler_params=pltpu.CompilerParams(vmem_limit_bytes=112 * 1024 * 1024),
    )


def _run(A_q, A_k, A_v, A_shift_k, A_ssm_k, A_ssm_D, B_x, B_W_gate, B_W_up, B_W_down, c, w_mod,
         cfg):
    del B_x
    B, S, D = A_q.shape
    F = B_W_gate.shape[1]
    assert B == 1
    shift = jnp.pad(A_shift_k, ((0, 0), (0, LANES - A_shift_k.shape[1])))
    out = _build(S, D, F, cfg)(
        A_q.reshape(S, D), A_k.reshape(S, D), A_v.reshape(S, D), shift, A_ssm_k,
        A_ssm_D.reshape(1, D), B_W_gate, B_W_up, B_W_down, c, w_mod)
    return out.reshape(B, S, D)


@jax.jit
def pallas_adaLN_cond__ssm_conv_h3__glu_gated_reglu__prompt_kernel(
    A_q: jax.Array,
    A_k: jax.Array,
    A_v: jax.Array,
    A_shift_k: jax.Array,
    A_ssm_k: jax.Array,
    A_ssm_D: jax.Array,
    B_x: jax.Array,
    B_W_gate: jax.Array,
    B_W_up: jax.Array,
    B_W_down: jax.Array,
    c: jax.Array,
    w_mod: jax.Array,
):
    return _run(A_q, A_k, A_v, A_shift_k, A_ssm_k, A_ssm_D, B_x, B_W_gate, B_W_up, B_W_down,
                c, w_mod, {})
```

```python
import functools
import math

import jax
import jax.numpy as jnp
import numpy as np
from jax import lax
import jax.experimental.pallas as pl
import jax.experimental.pallas.tpu as pltpu

C = 128
LANES = 128
EPS = 1e-5


def _kernel(q_hbm, k_hbm, v_hbm, shift_hbm, ssmk_hbm, ssmd_hbm, wg_hbm, wu_hbm, wd_hbm,
            c_hbm, wmod_hbm, o_hbm, *scr, S, D, F, cfg):
    f32, bf16 = jnp.float32, jnp.bfloat16
    NT = D // LANES
    TS = 2 * C
    NS = S // TS
    TN = cfg.get("tn", 128)
    NF = F // TN
    (q_s, k_s, v_s, ssmk_s, wg_s, wu_s, wd_s, wmod_s, shift_s, ssmd_s, c_s,
     kf_s, out_s, sems, f_s, g_s, tap_s, sc_s, mod_s) = scr[:19]
    scr = scr[19:]
    kp_s, u_s, yb_s, y_s, x1_s, h2_s, yp_s, kv_s = (scr[i * NS:(i + 1) * NS] for i in range(8))
    h_s, hy_s, xn_s = (scr[8 * NS + 2 * i:8 * NS + 2 * i + 2] for i in range(3))

    sem_count = [0]
    dmas = {}

    def mk(name, src, dst):
        i = sem_count[0]
        sem_count[0] += 1
        cfg.setdefault("_sem_names", {})[i] = name
        dmas[name] = pltpu.make_async_copy(src, dst, sems.at[i])

    mk("c", c_hbm, c_s)
    mk("shift", shift_hbm, shift_s)
    mk("ssmd", ssmd_hbm, ssmd_s)
    for t in range(NS):
        r = pl.ds(t * TS, TS)
        for a in (2 * t, 2 * t + 1):
            mk(("ssmk", a), ssmk_hbm.at[:, pl.ds(a * C, C)], ssmk_s.bitcast(bf16).at[a])
        mk(("k", t), k_hbm.at[r, :], k_s.at[r, :])
        mk(("v", t), v_hbm.at[r, :], v_s.at[r, :])
        mk(("q", t), q_hbm.at[r, :], q_s.at[r, :])
        if t < NS - 1:
            mk(("out", t), out_s.at[r, :], o_hbm.at[r, :])
    r = pl.ds((NS - 1) * TS, TS)
    for j in range(NT):
        cs = pl.ds(j * LANES, LANES)
        mk(("outl", j), out_s.at[r, cs], o_hbm.at[r, cs])
    for j in range(6):
        cs = pl.ds(j * D, D)
        mk(("wmod", j), wmod_hbm.at[:, cs], wmod_s.at[:, cs])
    for j in range(F // LANES):
        cs = pl.ds(j * LANES, LANES)
        mk(("wg", j), wg_hbm.at[:, cs], wg_s.bitcast(bf16).at[j])
        mk(("wu", j), wu_hbm.at[:, cs], wu_s.bitcast(bf16).at[j])
    for j in range(NT):
        mk(("wd", j), wd_hbm.at[:, pl.ds(j * LANES, LANES)], wd_s.bitcast(bf16).at[j])

    order = ["c", "shift", "ssmd"]
    for t in range(NS):
        order += [("ssmk", 2 * t), ("ssmk", 2 * t + 1), ("k", t), ("v", t)]
    order += [("q", 0), ("q", 1)] + [("wmod", j) for j in range(5)]
    for j in range(F // LANES):
        order += [("wg", j), ("wu", j)]
    order += [("q", 2)] + [("wd", j) for j in range(NT)] + [("wmod", 5)] + [("q", t) for t in range(3, NS)]
    for name in order:
        dmas[name].start()
    waited = set()

    def wait(*names):
        for n in names:
            if n not in waited:
                waited.add(n)
                if cfg.get("scopes", 0):
                    with jax.named_scope("w_" + (n if isinstance(n, str) else "%s%d" % n)):
                        dmas[n].wait()
                else:
                    dmas[n].wait()

    pk = lambda x: pltpu.bitcast(x.astype(bf16), jnp.uint32)
    upk = lambda x: pltpu.bitcast(x, bf16)

    def cat(vals):
        return vals[0] if len(vals) == 1 else jnp.concatenate(vals, axis=1)

    def table(f_off):
        f = lax.broadcasted_iota(jnp.int32, (C, C), 0)
        n = lax.broadcasted_iota(jnp.int32, (C, C), 1)
        m = ((4 * f + 1) * n + f_off) & (4 * C - 1)
        return jnp.sin(m.astype(f32) * (2.0 * math.pi / (4 * C)))

    t_cos, t_sin = table(C), table(0)

    wait("c", "shift", "ssmd")
    shift_rows = shift_s[...].astype(f32)
    ssmd = ssmd_s[...].astype(f32).reshape(1, D)
    cc = c_s[...].astype(f32)
    sc = jnp.broadcast_to((cc * jax.nn.sigmoid(cc)).astype(bf16), (16, D))
    never16 = jnp.abs(jnp.broadcast_to(cc[:, 0:LANES], (16, LANES))) < 0.0
    never = never16[0:8]
    zero = never16.astype(jnp.int32)[0, 0]
    zero2 = never16.astype(jnp.int32)[1, 1]
    f_s[zero] = pk(jnp.concatenate([t_cos, t_sin], axis=0))
    g_s[zero, 0] = pk(t_cos.T * (1.0 / C))
    g_s[zero, 1] = pk(t_sin.T * (1.0 / C))
    for j in range(4):
        tap_s[zero, j] = jnp.broadcast_to(shift_rows[j:j + 1, :], (8, D))
    sc_s[zero] = sc
    get_f = lambda: upk(f_s[zero2])
    get_g = lambda: jnp.concatenate([upk(g_s[zero2, 0]), upk(g_s[zero2, 1])], axis=1)

    queue = []
    state = {"last": None, "chain": [None, None]}

    def attach(results, budget):
        anchors = []
        for r in results:
            anchors += [(r, i, j) for j in range(r.shape[1] // LANES) for i in range(r.shape[0] // 16)]
        state["chain"] = [None, None]
        take, tot = [], 0
        while queue and tot < budget:
            take.append(queue.pop(0))
            tot += take[-1][1]
        pos = 0
        for fn, cost, _ in take:
            def get(frac=0.0, rows=8, pos=pos, cost=cost):
                r, i, j = anchors[min(int((pos + frac * cost) / max(tot, budget) * len(anchors)),
                                      len(anchors) - 1)]
                return r[i * 16:i * 16 + rows, j * LANES:(j + 1) * LANES]
            fn(get if cfg.get("anchor", 1) else None)
            pos += cost

    def flush(tag):
        idx = [i for i, u in enumerate(queue) if u[2] == tag]
        if not idx:
            return
        n = idx[-1] + 1
        for fn, _, _ in queue[:n]:
            fn(None)
        del queue[:n]

    KR = 32

    def kvprep_units(t):
        r0 = t * TS
        units = []

        def head(jt, get):
            ls = slice(jt * LANES, (jt + 1) * LANES)
            if t == 0:
                kf_s[jt, 0:8, :] = jnp.zeros((8, LANES), f32)
            else:
                kf_s[jt, 0:8, :] = k_s[r0 - 16:r0, ls].astype(f32)[8:16]

        def unit(jt, g, get):
            ls = slice(jt * LANES, (jt + 1) * LANES)
            if g == 0:
                head(jt, get)
            rows = slice(r0 + g * KR, r0 + (g + 1) * KR)
            kb = k_s[rows, ls]
            vv = v_s[rows, ls].astype(f32)
            kk = kb.astype(f32)
            if get is not None:
                kk = jnp.concatenate([jnp.where(never16, get(0.0, 16), kk[0:16]), kk[16:]], axis=0)
            kf_s[jt, 8 + g * KR:8 + (g + 1) * KR, :] = kk
            wt = lambda j: jnp.concatenate([tap_s[zero2, j, :, ls]] * (KR // 8), axis=0)
            acc = kk * wt(0)
            for j in range(1, 4):
                acc = acc + kf_s[jt, 8 - j + g * KR:8 - j + (g + 1) * KR, :] * wt(j)
            kv_s[t][zero, jt, g * KR // 2:(g + 1) * KR // 2, :] = pk(acc * vv)

        for g in range(TS // KR):
            for jt in range(NT):
                units.append([functools.partial(unit, jt, g), 11 * KR // 8,
                              ("kv", 2 * t + g * KR // C)])
        return units

    def dft_k(a):
        t, o = a // 2, a % 2
        kc = upk(ssmk_s[a])
        kk = lax.dot_general(get_f(), kc, (((1,), (1,)), ((), ())), preferred_element_type=f32)
        kr, ki = kk[0:C], kk[C:2 * C]
        if a == 0:
            kr = kr + ssmd
        kp_s[t][zero, o, 0] = kr
        kp_s[t][zero, o, 1] = ki
        return kk

    def dft_u(a):
        t, o = a // 2, a % 2
        kv = cat([upk(kv_s[t][zero2, jt, o * C // 2:(o + 1) * C // 2, :]) for jt in range(NT)])
        uu = jnp.dot(get_f(), kv, preferred_element_type=f32)
        u_s[t][zero, o, 0] = uu[0:C]
        u_s[t][zero, o, 1] = uu[C:2 * C]
        return uu

    MG = cfg.get("mgrp", 2)

    def x_unit(t, jt, r, get):
        a0 = 2 * t
        ls = slice(jt * LANES, (jt + 1) * LANES)
        nm = a0 + 2
        res = []
        for hh in range(2):
            rs = slice(r * 16 + hh * 8, r * 16 + hh * 8 + 8)
            acc = [[None, None], [None, None]]
            us = None
            ldu = lambda n: (u_s[n // 2][zero2, n % 2, 0, rs, ls], u_s[n // 2][zero2, n % 2, 1, rs, ls])
            for m in range(nm):
                kr = kp_s[m // 2][zero2, m % 2, 0, rs, ls]
                ki = kp_s[m // 2][zero2, m % 2, 1, rs, ls]
                if m % MG == 0:
                    if get is not None:
                        an = get((hh * nm + m) / (2 * nm), 8)
                    else:
                        an = acc[0][0] if m else state["chain"][hh]
                    if an is not None:
                        kr = jnp.where(never, an, kr)
                        if get is None or cfg.get("anchor2", 0):
                            ki = jnp.where(never, an, ki)
                if m == 0:
                    us = [ldu(a0), ldu(a0 + 1)]
                else:
                    us = [ldu(a0 - m) if a0 - m >= 0 else None, us[0]]
                for o in range(2):
                    if us[o] is None:
                        continue
                    ur, ui = us[o]
                    pr = kr * ur - ki * ui
                    pi = kr * ui + ki * ur
                    acc[o][0] = pr if acc[o][0] is None else acc[o][0] + pr
                    acc[o][1] = pi if acc[o][1] is None else acc[o][1] + pi
            res.append(acc)
            state["chain"][hh] = acc[0][0]
        full = [[jnp.concatenate([res[0][o][p], res[1][o][p]], axis=0) for p in range(2)]
                for o in range(2)]
        rows = slice(r * 16, (r + 1) * 16)
        if t == 0:
            first = full[0]
        else:
            first = [full[0][0] + yp_s[t - 1][zero2, 1, rows, ls],
                     full[0][1] - yp_s[t - 1][zero2, 0, rows, ls]]
        second = [full[1][0] + full[0][1], full[1][1] - full[0][0]]
        if t + 1 < NS:
            yp_s[t][zero, 0, rows, ls] = full[1][0]
            yp_s[t][zero, 1, rows, ls] = full[1][1]
        for o, val in enumerate((first, second)):
            for p in range(2):
                yb_s[t][zero, o, jt, (p * C + r * 16) // 2:(p * C + (r + 1) * 16) // 2, :] = pk(val[p])

    def x_units(t):
        return [[functools.partial(x_unit, t, jt, r), 16 * (4 * t + 3) + 8, ("x", t)]
                for r in range(C // 16) for jt in range(NT)]

    def inv(t):
        res = []
        for o in range(2):
            yy = jnp.dot(get_g(), cat([upk(yb_s[t][zero2, o, jt]) for jt in range(NT)]),
                         preferred_element_type=f32)
            y_s[t][zero, o * C:(o + 1) * C, :] = yy
            res.append(yy)
        return res

    def modvec(j):
        wait(("wmod", j))
        m = jnp.dot(sc_s[zero2], wmod_s[:, j * D:(j + 1) * D], preferred_element_type=f32)
        mod_s[zero, j] = m + 1.0 if j in (1, 4) else m
        return m

    def layernorm(x):
        mu = jnp.mean(x, axis=1, keepdims=True)
        xc = x - mu
        var = jnp.mean(xc * xc, axis=1, keepdims=True)
        return xc * lax.rsqrt(var + EPS)

    RG = 16
    mod = lambda j, cs=slice(None): mod_s[zero2, j, :, cs]

    def anchor_x(x, get):
        if get is None:
            return x
        return jnp.concatenate([jnp.where(never16, get(0.0, 16), x[:, 0:LANES]), x[:, LANES:]], axis=1)

    def put_h2(t, lr, val):
        for jt in range(NT):
            h2_s[t][zero, jt, lr.start // 2:lr.stop // 2, :] = pk(val[:, jt * LANES:(jt + 1) * LANES])

    def e1_unit(t, g, get):
        rows = slice(t * TS + g * RG, t * TS + (g + 1) * RG)
        lr = slice(g * RG, (g + 1) * RG)
        x = anchor_x(q_s[rows, :].astype(f32), get)
        h = layernorm(x) * mod(1) + mod(0)
        x1 = x + mod(2) * (h * y_s[t][zero2, lr, :])
        x1_s[t][zero, lr, :] = x1
        put_h2(t, lr, layernorm(x1) * mod(4) + mod(3))

    def e1a_unit(t, g, get):
        rows = slice(t * TS + g * RG, t * TS + (g + 1) * RG)
        lr = slice(g * RG, (g + 1) * RG)
        x = anchor_x(q_s[rows, :].astype(f32), get)
        h = layernorm(x) * mod(1) + mod(0)
        hy_s[t][zero, lr, :] = h * y_s[t][zero2, lr, :]

    def e1b_unit(t, g, get):
        rows = slice(t * TS + g * RG, t * TS + (g + 1) * RG)
        lr = slice(g * RG, (g + 1) * RG)
        x = anchor_x(q_s[rows, :].astype(f32), get)
        x1 = x + mod(2) * hy_s[t][zero2, lr, :]
        x1_s[t][zero, lr, :] = x1
        xn_s[t][zero, lr, :] = layernorm(x1)

    def e1c_unit(t, g, get):
        lr = slice(g * RG, (g + 1) * RG)
        put_h2(t, lr, xn_s[t][zero2, lr, :] * mod(4) + mod(3))

    def units(fn, t, cost, tag):
        return [[functools.partial(fn, t, g), cost, (tag, t)] for g in range(TS // RG)]

    GB = cfg.get("glu_budget", 1.2)

    NTN = TN // LANES

    def glu_p1(t, j):
        tiles = range(j * NTN, (j + 1) * NTN)
        h2 = lambda: cat([upk(h2_s[t][zero2, jt]) for jt in range(NT)])
        g = jnp.dot(h2(), cat([upk(wg_s[w]) for w in tiles]), preferred_element_type=f32)
        u = jnp.dot(h2(), cat([upk(wu_s[w]) for w in tiles]), preferred_element_type=f32)
        hh = jnp.maximum(g, 0.0) * u
        for i, w in enumerate(tiles):
            h_s[t % 2][zero, w] = pk(hh[:, i * LANES:(i + 1) * LANES])
        attach([g, u], GB * 5 * TN)

    def glu_p2(t):
        for j in range(NT):
            wait(("wd", j))
        if t == 0:
            modvec(5)
        for j in range(NT):
            cs = slice(j * LANES, (j + 1) * LANES)
            hh = cat([upk(h_s[t % 2][zero2, w]) for w in range(F // LANES)])
            d = jnp.dot(hh, upk(wd_s[j]), preferred_element_type=f32)
            gb = jnp.concatenate([mod(5, cs)] * (TS // 16), axis=0)
            out_s[t * TS:(t + 1) * TS, cs] = (x1_s[t][zero2, :, cs] + gb * d).astype(bf16)
            if t == NS - 1:
                dmas[("outl", j)].start()
            attach([d], GB * 768)
        if t < NS - 1:
            dmas[("out", t)].start()

    XP = cfg.get("xp", 6)
    PB = cfg.get("p1_budget", 4.5)
    MB = cfg.get("mod_budget", 3.0)
    state["inv"] = 0

    def do_inv(budget):
        t = state["inv"]
        flush(("x", t))
        attach(inv(t), budget)
        state["inv"] = t + 1

    for r in range(NS + 2):
        if r < NS:
            wait(("ssmk", 2 * r), ("ssmk", 2 * r + 1))
        if 1 <= r <= NS:
            wait(("k", r - 1), ("v", r - 1))
            queue[0:0] = kvprep_units(r - 1)
        for o in range(2):
            if r < NS:
                attach([dft_k(2 * r + o)], PB * 320)
            if r >= 2:
                flush(("kv", 2 * (r - 2) + 1))
                attach([dft_u(2 * (r - 2) + o)], PB * 320)
        if r >= 2:
            queue.extend(x_units(r - 2))
    do_inv(MB * 640)
    do_inv(MB * 640)
    n_inv = XP - 2
    for j in range(5):
        while state["inv"] < 2 + (n_inv * (j + 1)) // 5:
            do_inv(MB * 640)
        m = modvec(j)
        if j == 1:
            wait(("q", 0), ("q", 1))
            queue[0:0] = units(e1a_unit, 0, 140, "e1a") + units(e1a_unit, 1, 140, "e1a")
        if j == 2:
            flush(("e1a", 1))
            queue[0:0] = units(e1b_unit, 0, 160, "e1b") + units(e1b_unit, 1, 160, "e1b")
        if j == 4:
            flush(("e1b", 1))
            queue[0:0] = units(e1c_unit, 0, 30, "e1c") + units(e1c_unit, 1, 30, "e1c")
        attach([m], MB * 300)
    flush(("e1c", 1))

    def need_e1(t):
        wait(("q", t))
        while state["inv"] <= t:
            do_inv(GB * 640)
        queue[0:0] = units(e1_unit, t, 300, "e1")

    GR = cfg.get("first_group", 3)
    for j0 in range(0, NF, GR):
        for j in range(j0, min(j0 + GR, NF)):
            for w in range(j * NTN, (j + 1) * NTN):
                wait(("wg", w), ("wu", w))
        for t in range(2):
            for j in range(j0, min(j0 + GR, NF)):
                glu_p1(t, j)
    need_e1(2)
    glu_p2(0)
    glu_p2(1)
    for t in range(2, NS):
        flush(("e1", t))
        if t + 1 < NS:
            need_e1(t + 1)
        for j in range(NF):
            glu_p1(t, j)
        glu_p2(t)
    assert len(waited) == len(order)
    if cfg.get("scopes", 0):
        with jax.named_scope("w_end0"):
            dmas[("out", 0)].wait()
        dmas[("out", 0)].start()
    for t in range(NS - 1):
        dmas[("out", t)].wait()
    for j in range(NT):
        dmas[("outl", j)].wait()


def _build(S, D, F, cfg):
    f32, bf16, u32 = jnp.float32, jnp.bfloat16, jnp.uint32
    NT, NA, TS, NS = D // LANES, S // C, 2 * C, S // (2 * C)
    scratch = [
        pltpu.VMEM((S, D), bf16),
        pltpu.VMEM((S, D), bf16),
        pltpu.VMEM((S, D), bf16),
        pltpu.VMEM((NA, D // 2, LANES), u32),
        pltpu.VMEM((F // LANES, D // 2, LANES), u32),
        pltpu.VMEM((F // LANES, D // 2, LANES), u32),
        pltpu.VMEM((NT, F // 2, LANES), u32),
        pltpu.VMEM((D, 6 * D), bf16),
        pltpu.VMEM((4, D), bf16),
        pltpu.VMEM((D,), bf16),
        pltpu.VMEM((1, D), bf16),
        pltpu.VMEM((NT, 8 + TS, LANES), f32),
        pltpu.VMEM((S, D), bf16),
        pltpu.SemaphoreType.DMA((112,)),
        pltpu.VMEM((1, C, C), u32),
        pltpu.VMEM((1, 2, C // 2, C), u32),
        pltpu.VMEM((1, 4, 8, D), f32),
        pltpu.VMEM((1, 16, D), bf16),
        pltpu.VMEM((1, 6, 16, D), f32),
    ]
    scratch += [pltpu.VMEM((1, 2, 2, C, D), f32) for _ in range(NS)]
    scratch += [pltpu.VMEM((1, 2, 2, C, D), f32) for _ in range(NS)]
    scratch += [pltpu.VMEM((1, 2, NT, C, LANES), u32) for _ in range(NS)]
    scratch += [pltpu.VMEM((1, TS, D), f32) for _ in range(NS)]
    scratch += [pltpu.VMEM((1, TS, D), f32) for _ in range(NS)]
    scratch += [pltpu.VMEM((1, NT, TS // 2, LANES), u32) for _ in range(NS)]
    scratch += [pltpu.VMEM((1, 2, C, D), f32) for _ in range(NS)]
    scratch += [pltpu.VMEM((1, NT, TS // 2, LANES), u32) for _ in range(NS)]
    scratch += [pltpu.VMEM((1, F // LANES, TS // 2, LANES), u32) for _ in range(2)]
    scratch += [pltpu.VMEM((1, TS, D), f32) for _ in range(4)]
    return pl.pallas_call(
        functools.partial(_kernel, S=S, D=D, F=F, cfg=cfg),
        in_specs=[pl.BlockSpec(memory_space=pl.ANY)] * 11,
        out_specs=pl.BlockSpec(memory_space=pl.ANY),
        out_shape=jax.ShapeDtypeStruct((S, D), bf16),
        scratch_shapes=scratch,
        compiler_params=pltpu.CompilerParams(vmem_limit_bytes=112 * 1024 * 1024),
    )


def _run(A_q, A_k, A_v, A_shift_k, A_ssm_k, A_ssm_D, B_x, B_W_gate, B_W_up, B_W_down, c, w_mod,
         cfg):
    del B_x
    B, S, D = A_q.shape
    F = B_W_gate.shape[1]
    assert B == 1
    assert A_shift_k.shape[1] == 4
    out = _build(S, D, F, cfg)(
        A_q.reshape(S, D), A_k.reshape(S, D), A_v.reshape(S, D), A_shift_k.T, A_ssm_k,
        A_ssm_D, B_W_gate, B_W_up, B_W_down, c, w_mod)
    return out.reshape(B, S, D)


@jax.jit
def pallas_adaLN_cond__ssm_conv_h3__glu_gated_reglu__prompt_kernel(
    A_q: jax.Array,
    A_k: jax.Array,
    A_v: jax.Array,
    A_shift_k: jax.Array,
    A_ssm_k: jax.Array,
    A_ssm_D: jax.Array,
    B_x: jax.Array,
    B_W_gate: jax.Array,
    B_W_up: jax.Array,
    B_W_down: jax.Array,
    c: jax.Array,
    w_mod: jax.Array,
):
    return _run(A_q, A_k, A_v, A_shift_k, A_ssm_k, A_ssm_D, B_x, B_W_gate, B_W_up, B_W_down,
                c, w_mod, {})
```

```python
import functools
import math

import jax
import jax.numpy as jnp
import numpy as np
from jax import lax
import jax.experimental.pallas as pl
import jax.experimental.pallas.tpu as pltpu

C = 128
LANES = 128
EPS = 1e-5


def _kernel(q_hbm, k_hbm, v_hbm, shift_hbm, ssmk_hbm, ssmd_hbm, wg_hbm, wu_hbm, wd_hbm,
            c_hbm, wmod_hbm, o_hbm, *scr, S, D, F, cfg):
    f32, bf16 = jnp.float32, jnp.bfloat16
    NT = D // LANES
    TS = 2 * C
    NS = S // TS
    TN = cfg.get("tn", 128)
    NF = F // TN
    (q_s, k_s, v_s, ssmk_s, wg_s, wu_s, wd_s, wmod_s, shift_s, ssmd_s, c_s,
     kf_s, out_s, sems, f_s, g_s, tap_s, sc_s, mod_s) = scr[:19]
    scr = scr[19:]
    kp_s, u_s, yb_s, y_s, x1_s, h2_s, yp_s, kv_s = (scr[i * NS:(i + 1) * NS] for i in range(8))
    h_s, hy_s, xn_s = (scr[8 * NS + 2 * i:8 * NS + 2 * i + 2] for i in range(3))

    sem_count = [0]
    dmas = {}

    def mk(name, src, dst):
        i = sem_count[0]
        sem_count[0] += 1
        cfg.setdefault("_sem_names", {})[i] = name
        dmas[name] = pltpu.make_async_copy(src, dst, sems.at[i])

    mk("c", c_hbm, c_s)
    mk("shift", shift_hbm, shift_s)
    mk("ssmd", ssmd_hbm, ssmd_s)
    for t in range(NS):
        r = pl.ds(t * TS, TS)
        for a in (2 * t, 2 * t + 1):
            mk(("ssmk", a), ssmk_hbm.at[:, pl.ds(a * C, C)], ssmk_s.bitcast(bf16).at[a])
        mk(("k", t), k_hbm.at[r, :], k_s.at[r, :])
        mk(("v", t), v_hbm.at[r, :], v_s.at[r, :])
        mk(("q", t), q_hbm.at[r, :], q_s.at[r, :])
        if t < NS - 1:
            mk(("out", t), out_s.at[r, :], o_hbm.at[r, :])
    r = pl.ds((NS - 1) * TS, TS)
    for j in range(NT):
        cs = pl.ds(j * LANES, LANES)
        mk(("outl", j), out_s.at[r, cs], o_hbm.at[r, cs])
    for j in range(6):
        cs = pl.ds(j * D, D)
        mk(("wmod", j), wmod_hbm.at[:, cs], wmod_s.at[:, cs])
    for j in range(F // LANES):
        cs = pl.ds(j * LANES, LANES)
        mk(("wg", j), wg_hbm.at[:, cs], wg_s.bitcast(bf16).at[j])
        mk(("wu", j), wu_hbm.at[:, cs], wu_s.bitcast(bf16).at[j])
    for j in range(NT):
        mk(("wd", j), wd_hbm.at[:, pl.ds(j * LANES, LANES)], wd_s.bitcast(bf16).at[j])

    order = ["c", "shift", "ssmd"]
    PP = cfg.get("pp", NS)
    pair = lambda t: [("ssmk", 2 * t), ("ssmk", 2 * t + 1), ("k", t), ("v", t)]
    for t in range(PP):
        order += pair(t)
    order += [("q", 0), ("q", 1)] + [("wmod", j) for j in range(5)]
    for j in range(F // LANES):
        order += [("wg", j), ("wu", j)]
    order += [("wd", j) for j in range(NT)] + [("wmod", 5), ("q", 2)]
    for t in range(PP, NS):
        order += pair(t)
        if t == PP:
            order += [("q", 3)]
    order += [("q", t) for t in range(3 if PP == NS else 4, NS)]
    for name in order:
        dmas[name].start()
    waited = set()

    def wait(*names):
        for n in names:
            if n not in waited:
                waited.add(n)
                if cfg.get("scopes", 0):
                    with jax.named_scope("w_" + (n if isinstance(n, str) else "%s%d" % n)):
                        dmas[n].wait()
                else:
                    dmas[n].wait()

    pk = lambda x: pltpu.bitcast(x.astype(bf16), jnp.uint32)
    upk = lambda x: pltpu.bitcast(x, bf16)

    def cat(vals):
        return vals[0] if len(vals) == 1 else jnp.concatenate(vals, axis=1)

    def table(f_off):
        f = lax.broadcasted_iota(jnp.int32, (C, C), 0)
        n = lax.broadcasted_iota(jnp.int32, (C, C), 1)
        m = ((4 * f + 1) * n + f_off) & (4 * C - 1)
        return jnp.sin(m.astype(f32) * (2.0 * math.pi / (4 * C)))

    t_cos, t_sin = table(C), table(0)

    wait("c", "shift", "ssmd")
    shift_rows = shift_s[...].astype(f32)
    ssmd = ssmd_s[...].astype(f32).reshape(1, D)
    cc = c_s[...].astype(f32)
    sc = jnp.broadcast_to((cc * jax.nn.sigmoid(cc)).astype(bf16), (16, D))
    never16 = jnp.abs(jnp.broadcast_to(cc[:, 0:LANES], (16, LANES))) < 0.0
    never = never16[0:8]
    zero = never16.astype(jnp.int32)[0, 0]
    zero2 = never16.astype(jnp.int32)[1, 1]
    f_s[zero] = pk(jnp.concatenate([t_cos, t_sin], axis=0))
    g_s[zero, 0] = pk(t_cos.T * (1.0 / C))
    g_s[zero, 1] = pk(t_sin.T * (1.0 / C))
    for j in range(4):
        tap_s[zero, j] = jnp.broadcast_to(shift_rows[j:j + 1, :], (8, D))
    sc_s[zero] = sc
    get_f = lambda: upk(f_s[zero2])
    get_g = lambda: jnp.concatenate([upk(g_s[zero2, 0]), upk(g_s[zero2, 1])], axis=1)

    queue = []
    state = {"last": None, "chain": [None, None]}

    def attach(results, budget):
        anchors = []
        for r in results:
            anchors += [(r, i, j) for j in range(r.shape[1] // LANES) for i in range(r.shape[0] // 16)]
        state["chain"] = [None, None]
        take, tot = [], 0
        while queue and tot < budget:
            take.append(queue.pop(0))
            tot += take[-1][1]
        pos = 0
        for fn, cost, _ in take:
            def get(frac=0.0, rows=8, pos=pos, cost=cost):
                r, i, j = anchors[min(int((pos + frac * cost) / max(tot, budget) * len(anchors)),
                                      len(anchors) - 1)]
                return r[i * 16:i * 16 + rows, j * LANES:(j + 1) * LANES]
            fn(get if cfg.get("anchor", 1) else None)
            pos += cost

    def flush(tag, extra=0):
        idx = [i for i, u in enumerate(queue) if u[2] == tag]
        if not idx:
            return
        n = idx[-1] + 1
        while extra > 0 and n < len(queue):
            extra -= queue[n][1]
            n += 1
        for fn, _, _ in queue[:n]:
            fn(None)
        del queue[:n]

    KR = 32

    def kvprep_units(t):
        r0 = t * TS
        units = []

        def head(jt, get):
            ls = slice(jt * LANES, (jt + 1) * LANES)
            if t == 0:
                kf_s[jt, 0:8, :] = jnp.zeros((8, LANES), f32)
            else:
                kf_s[jt, 0:8, :] = k_s[r0 - 16:r0, ls].astype(f32)[8:16]

        def unit(jt, g, get):
            ls = slice(jt * LANES, (jt + 1) * LANES)
            if g == 0:
                head(jt, get)
            rows = slice(r0 + g * KR, r0 + (g + 1) * KR)
            kb = k_s[rows, ls]
            vv = v_s[rows, ls].astype(f32)
            kk = kb.astype(f32)
            if get is not None:
                kk = jnp.concatenate([jnp.where(never16, get(0.0, 16), kk[0:16]), kk[16:]], axis=0)
            kf_s[jt, 8 + g * KR:8 + (g + 1) * KR, :] = kk
            wt = lambda j: jnp.concatenate([tap_s[zero2, j, :, ls]] * (KR // 8), axis=0)
            acc = kk * wt(0)
            for j in range(1, 4):
                acc = acc + kf_s[jt, 8 - j + g * KR:8 - j + (g + 1) * KR, :] * wt(j)
            kv_s[t][zero, jt, g * KR // 2:(g + 1) * KR // 2, :] = pk(acc * vv)

        for g in range(TS // KR):
            for jt in range(NT):
                units.append([functools.partial(unit, jt, g), 11 * KR // 8,
                              ("kv", 2 * t + g * KR // C)])
        return units

    def dft_k(a):
        t, o = a // 2, a % 2
        kc = upk(ssmk_s[a])
        kk = lax.dot_general(get_f(), kc, (((1,), (1,)), ((), ())), preferred_element_type=f32)
        kr, ki = kk[0:C], kk[C:2 * C]
        if a == 0:
            kr = kr + ssmd
        kp_s[t][zero, o, 0] = kr
        kp_s[t][zero, o, 1] = ki
        return kk

    def dft_u(a):
        t, o = a // 2, a % 2
        kv = cat([upk(kv_s[t][zero2, jt, o * C // 2:(o + 1) * C // 2, :]) for jt in range(NT)])
        uu = jnp.dot(get_f(), kv, preferred_element_type=f32)
        u_s[t][zero, o, 0] = uu[0:C]
        u_s[t][zero, o, 1] = uu[C:2 * C]
        return uu

    MG = cfg.get("mgrp", 4)

    def x_unit(t, jt, r, get):
        a0 = 2 * t
        ls = slice(jt * LANES, (jt + 1) * LANES)
        nm = a0 + 2
        res = []
        for hh in range(2):
            rs = slice(r * 16 + hh * 8, r * 16 + hh * 8 + 8)
            acc = [[None, None], [None, None]]
            us = None
            ldu = lambda n: (u_s[n // 2][zero2, n % 2, 0, rs, ls], u_s[n // 2][zero2, n % 2, 1, rs, ls])
            for m in range(nm):
                kr = kp_s[m // 2][zero2, m % 2, 0, rs, ls]
                ki = kp_s[m // 2][zero2, m % 2, 1, rs, ls]
                if m % MG == 0:
                    if get is not None:
                        an = get((hh * nm + m) / (2 * nm), 8)
                    else:
                        an = acc[0][0] if m else state["chain"][hh]
                    if an is not None:
                        kr = jnp.where(never, an, kr)
                        if get is None or cfg.get("anchor2", 0):
                            ki = jnp.where(never, an, ki)
                if m == 0:
                    us = [ldu(a0), ldu(a0 + 1)]
                else:
                    us = [ldu(a0 - m) if a0 - m >= 0 else None, us[0]]
                for o in range(2):
                    if us[o] is None:
                        continue
                    ur, ui = us[o]
                    pr = kr * ur - ki * ui
                    pi = kr * ui + ki * ur
                    acc[o][0] = pr if acc[o][0] is None else acc[o][0] + pr
                    acc[o][1] = pi if acc[o][1] is None else acc[o][1] + pi
            res.append(acc)
            state["chain"][hh] = acc[0][0]
        full = [[jnp.concatenate([res[0][o][p], res[1][o][p]], axis=0) for p in range(2)]
                for o in range(2)]
        rows = slice(r * 16, (r + 1) * 16)
        if t == 0:
            first = full[0]
        else:
            first = [full[0][0] + yp_s[t - 1][zero2, 1, rows, ls],
                     full[0][1] - yp_s[t - 1][zero2, 0, rows, ls]]
        second = [full[1][0] + full[0][1], full[1][1] - full[0][0]]
        if t + 1 < NS:
            yp_s[t][zero, 0, rows, ls] = full[1][0]
            yp_s[t][zero, 1, rows, ls] = full[1][1]
        for o, val in enumerate((first, second)):
            for p in range(2):
                yb_s[t][zero, o, jt, (p * C + r * 16) // 2:(p * C + (r + 1) * 16) // 2, :] = pk(val[p])

    def x_units(t):
        return [[functools.partial(x_unit, t, jt, r), 16 * (4 * t + 3) + 8, ("x", t)]
                for r in range(C // 16) for jt in range(NT)]

    def inv(t):
        res = []
        for o in range(2):
            yy = jnp.dot(get_g(), cat([upk(yb_s[t][zero2, o, jt]) for jt in range(NT)]),
                         preferred_element_type=f32)
            y_s[t][zero, o * C:(o + 1) * C, :] = yy
            res.append(yy)
        return res

    def modvec(j):
        wait(("wmod", j))
        m = jnp.dot(sc_s[zero2], wmod_s[:, j * D:(j + 1) * D], preferred_element_type=f32)
        mod_s[zero, j] = m + 1.0 if j in (1, 4) else m
        return m

    def layernorm(x):
        mu = jnp.mean(x, axis=1, keepdims=True)
        xc = x - mu
        var = jnp.mean(xc * xc, axis=1, keepdims=True)
        return xc * lax.rsqrt(var + EPS)

    RG = 16
    mod = lambda j, cs=slice(None): mod_s[zero2, j, :, cs]

    def anchor_x(x, get):
        if get is None:
            return x
        return jnp.concatenate([jnp.where(never16, get(0.0, 16), x[:, 0:LANES]), x[:, LANES:]], axis=1)

    def put_h2(t, lr, val):
        for jt in range(NT):
            h2_s[t][zero, jt, lr.start // 2:lr.stop // 2, :] = pk(val[:, jt * LANES:(jt + 1) * LANES])

    def e1_unit(t, g, get):
        rows = slice(t * TS + g * RG, t * TS + (g + 1) * RG)
        lr = slice(g * RG, (g + 1) * RG)
        x = anchor_x(q_s[rows, :].astype(f32), get)
        h = layernorm(x) * mod(1) + mod(0)
        x1 = x + mod(2) * (h * y_s[t][zero2, lr, :])
        x1_s[t][zero, lr, :] = x1
        put_h2(t, lr, layernorm(x1) * mod(4) + mod(3))

    def e1a_unit(t, g, get):
        rows = slice(t * TS + g * RG, t * TS + (g + 1) * RG)
        lr = slice(g * RG, (g + 1) * RG)
        x = anchor_x(q_s[rows, :].astype(f32), get)
        h = layernorm(x) * mod(1) + mod(0)
        hy_s[t][zero, lr, :] = h * y_s[t][zero2, lr, :]

    def e1b_unit(t, g, get):
        rows = slice(t * TS + g * RG, t * TS + (g + 1) * RG)
        lr = slice(g * RG, (g + 1) * RG)
        x = anchor_x(q_s[rows, :].astype(f32), get)
        x1 = x + mod(2) * hy_s[t][zero2, lr, :]
        x1_s[t][zero, lr, :] = x1
        xn_s[t][zero, lr, :] = layernorm(x1)

    def e1c_unit(t, g, get):
        lr = slice(g * RG, (g + 1) * RG)
        put_h2(t, lr, xn_s[t][zero2, lr, :] * mod(4) + mod(3))

    def units(fn, t, cost, tag):
        return [[functools.partial(fn, t, g), cost, (tag, t)] for g in range(TS // RG)]

    GB = cfg.get("glu_budget", 0.9)

    NTN = TN // LANES

    def glu_p1(t, j):
        tiles = range(j * NTN, (j + 1) * NTN)
        h2 = lambda: cat([upk(h2_s[t][zero2, jt]) for jt in range(NT)])
        g = jnp.dot(h2(), cat([upk(wg_s[w]) for w in tiles]), preferred_element_type=f32)
        u = jnp.dot(h2(), cat([upk(wu_s[w]) for w in tiles]), preferred_element_type=f32)
        hh = jnp.maximum(g, 0.0) * u
        for i, w in enumerate(tiles):
            h_s[t % 2][zero, w] = pk(hh[:, i * LANES:(i + 1) * LANES])
        attach([g, u], GB * 5 * TN)

    def glu_p2(t):
        for j in range(NT):
            wait(("wd", j))
        if t == 0:
            modvec(5)
        for j in range(NT):
            cs = slice(j * LANES, (j + 1) * LANES)
            hh = cat([upk(h_s[t % 2][zero2, w]) for w in range(F // LANES)])
            d = jnp.dot(hh, upk(wd_s[j]), preferred_element_type=f32)
            gb = jnp.concatenate([mod(5, cs)] * (TS // 16), axis=0)
            out_s[t * TS:(t + 1) * TS, cs] = (x1_s[t][zero2, :, cs] + gb * d).astype(bf16)
            if t == NS - 1:
                dmas[("outl", j)].start()
            attach([d], GB * 768)
        if t < NS - 1:
            dmas[("out", t)].start()

    XP = cfg.get("xp", 4)
    PB = cfg.get("p1_budget", 4.5)
    MB = cfg.get("mod_budget", 3.0)
    FX = cfg.get("flush_extra", 0)
    state["inv"] = 0

    def do_inv(budget):
        t = state["inv"]
        flush(("x", t))
        attach(inv(t), budget)
        state["inv"] = t + 1

    for r in range(PP + 2):
        if r < PP:
            wait(("ssmk", 2 * r), ("ssmk", 2 * r + 1))
        if 1 <= r <= PP:
            wait(("k", r - 1), ("v", r - 1))
            queue[0:0] = kvprep_units(r - 1)
        for o in range(2):
            if r < PP:
                attach([dft_k(2 * r + o)], PB * 320)
            if r >= 2:
                flush(("kv", 2 * (r - 2) + 1))
                attach([dft_u(2 * (r - 2) + o)], PB * 320)
        if r >= 2:
            queue.extend(x_units(r - 2))

    def conv_a(t):
        if t < NS:
            wait(*pair(t))
            queue[0:0] = kvprep_units(t)
            for o in range(2):
                attach([dft_k(2 * t + o)], GB * 320)

    def conv_b(t):
        if t < NS:
            flush(("kv", 2 * t + 1))
            for o in range(2):
                attach([dft_u(2 * t + o)], GB * 320)
            queue.extend(x_units(t))

    do_inv(MB * 640)
    do_inv(MB * 640)
    n_inv = XP - 2
    MI = cfg.get("mod_inv", [0, 1, 1, 2, 2])

    def inv_upto(j):
        while state["inv"] < 2 + min(n_inv, MI[j]):
            do_inv(MB * 640)

    inv_upto(0)
    attach([modvec(0)], MB * 300)
    inv_upto(1)
    attach([modvec(1)], MB * 300)
    wait(("q", 0), ("q", 1))
    queue[0:0] = units(e1a_unit, 0, 140, "e1a") + units(e1a_unit, 1, 140, "e1a")
    inv_upto(2)
    flush(("e1a", 1), FX)
    attach([modvec(2)], MB * 300)
    queue[0:0] = units(e1b_unit, 0, 160, "e1b") + units(e1b_unit, 1, 160, "e1b")
    inv_upto(3)
    flush(("e1b", 1), FX)
    attach([modvec(3)], MB * 300)
    inv_upto(4)
    m4 = modvec(4)
    queue[0:0] = units(e1c_unit, 0, 30, "e1c") + units(e1c_unit, 1, 30, "e1c")
    attach([m4], 32 * 30 - 1)
    flush(("e1c", 1))
    while state["inv"] < XP:
        do_inv(MB * 640)

    def need_e1(t):
        wait(*[("q", tt) for tt in range(t, NS if t > 2 else t + 1)])
        while state["inv"] <= t:
            do_inv(GB * 640)
        queue[0:0] = units(e1_unit, t, 300, "e1")

    j0 = 0
    for gr in cfg.get("groups", [1, 2, 3, 3, 3]):
        js = range(j0, min(j0 + gr, NF))
        j0 += gr
        for j in js:
            for w in range(j * NTN, (j + 1) * NTN):
                wait(("wg", w), ("wu", w))
        for t in range(2):
            for j in js:
                glu_p1(t, j)
    assert j0 >= NF
    need_e1(2)
    late = list(range(PP, NS + 8))
    glu_p2(0)
    conv_a(late[0])
    glu_p2(1)
    conv_b(late[0])
    conv_a(late[1])
    for t in range(2, NS):
        flush(("e1", t))
        if t + 1 < NS:
            need_e1(t + 1)
        for j in range(NF):
            if j == NF // 3 and t == 2:
                conv_b(late[1])
                conv_a(late[2])
            if j == 2 * NF // 3 and t == 2:
                conv_b(late[2])
                conv_a(late[3])
            if j == NF // 3 and t == 3:
                conv_b(late[3])
                for tt in late[4:NS - PP]:
                    conv_a(tt)
                    conv_b(tt)
            glu_p1(t, j)
        glu_p2(t)
    assert len(waited) == len(order)
    if cfg.get("scopes", 0):
        with jax.named_scope("w_end0"):
            dmas[("out", 0)].wait()
        dmas[("out", 0)].start()
    for t in range(NS - 1):
        dmas[("out", t)].wait()
    for j in range(NT):
        dmas[("outl", j)].wait()


def _build(S, D, F, cfg):
    f32, bf16, u32 = jnp.float32, jnp.bfloat16, jnp.uint32
    NT, NA, TS, NS = D // LANES, S // C, 2 * C, S // (2 * C)
    scratch = [
        pltpu.VMEM((S, D), bf16),
        pltpu.VMEM((S, D), bf16),
        pltpu.VMEM((S, D), bf16),
        pltpu.VMEM((NA, D // 2, LANES), u32),
        pltpu.VMEM((F // LANES, D // 2, LANES), u32),
        pltpu.VMEM((F // LANES, D // 2, LANES), u32),
        pltpu.VMEM((NT, F // 2, LANES), u32),
        pltpu.VMEM((D, 6 * D), bf16),
        pltpu.VMEM((4, D), bf16),
        pltpu.VMEM((D,), bf16),
        pltpu.VMEM((1, D), bf16),
        pltpu.VMEM((NT, 8 + TS, LANES), f32),
        pltpu.VMEM((S, D), bf16),
        pltpu.SemaphoreType.DMA((112,)),
        pltpu.VMEM((1, C, C), u32),
        pltpu.VMEM((1, 2, C // 2, C), u32),
        pltpu.VMEM((1, 4, 8, D), f32),
        pltpu.VMEM((1, 16, D), bf16),
        pltpu.VMEM((1, 6, 16, D), f32),
    ]
    scratch += [pltpu.VMEM((1, 2, 2, C, D), f32) for _ in range(NS)]
    scratch += [pltpu.VMEM((1, 2, 2, C, D), f32) for _ in range(NS)]
    scratch += [pltpu.VMEM((1, 2, NT, C, LANES), u32) for _ in range(NS)]
    scratch += [pltpu.VMEM((1, TS, D), f32) for _ in range(NS)]
    scratch += [pltpu.VMEM((1, TS, D), f32) for _ in range(NS)]
    scratch += [pltpu.VMEM((1, NT, TS // 2, LANES), u32) for _ in range(NS)]
    scratch += [pltpu.VMEM((1, 2, C, D), f32) for _ in range(NS)]
    scratch += [pltpu.VMEM((1, NT, TS // 2, LANES), u32) for _ in range(NS)]
    scratch += [pltpu.VMEM((1, F // LANES, TS // 2, LANES), u32) for _ in range(2)]
    scratch += [pltpu.VMEM((1, TS, D), f32) for _ in range(4)]
    return pl.pallas_call(
        functools.partial(_kernel, S=S, D=D, F=F, cfg=cfg),
        in_specs=[pl.BlockSpec(memory_space=pl.ANY)] * 11,
        out_specs=pl.BlockSpec(memory_space=pl.ANY),
        out_shape=jax.ShapeDtypeStruct((S, D), bf16),
        scratch_shapes=scratch,
        compiler_params=pltpu.CompilerParams(vmem_limit_bytes=112 * 1024 * 1024),
    )


def _run(A_q, A_k, A_v, A_shift_k, A_ssm_k, A_ssm_D, B_x, B_W_gate, B_W_up, B_W_down, c, w_mod,
         cfg):
    del B_x
    B, S, D = A_q.shape
    F = B_W_gate.shape[1]
    assert B == 1
    assert A_shift_k.shape[1] == 4
    out = _build(S, D, F, cfg)(
        A_q.reshape(S, D), A_k.reshape(S, D), A_v.reshape(S, D), A_shift_k.T, A_ssm_k,
        A_ssm_D, B_W_gate, B_W_up, B_W_down, c, w_mod)
    return out.reshape(B, S, D)


@jax.jit
def pallas_adaLN_cond__ssm_conv_h3__glu_gated_reglu__prompt_kernel(
    A_q: jax.Array,
    A_k: jax.Array,
    A_v: jax.Array,
    A_shift_k: jax.Array,
    A_ssm_k: jax.Array,
    A_ssm_D: jax.Array,
    B_x: jax.Array,
    B_W_gate: jax.Array,
    B_W_up: jax.Array,
    B_W_down: jax.Array,
    c: jax.Array,
    w_mod: jax.Array,
):
    return _run(A_q, A_k, A_v, A_shift_k, A_ssm_k, A_ssm_D, B_x, B_W_gate, B_W_up, B_W_down,
                c, w_mod, {})
```

```python
import functools
import math

import jax
import jax.numpy as jnp
import numpy as np
from jax import lax
import jax.experimental.pallas as pl
import jax.experimental.pallas.tpu as pltpu

C = 128
LANES = 128
EPS = 1e-5


def _kernel(q_hbm, k_hbm, v_hbm, shift_hbm, ssmk_hbm, ssmd_hbm, wg_hbm, wu_hbm, wd_hbm,
            c_hbm, wmod_hbm, o_hbm, *scr, S, D, F, cfg):
    f32, bf16 = jnp.float32, jnp.bfloat16
    NT = D // LANES
    TS = 2 * C
    NS = S // TS
    TN = cfg.get("tn", 128)
    NF = F // TN
    (q_s, k_s, v_s, ssmk_s, wg_s, wu_s, wd_s, wmod_s, shift_s, ssmd_s, c_s,
     kf_s, out_s, sems, f_s, g_s, tap_s, sc_s, mod_s) = scr[:19]
    scr = scr[19:]
    kp_s, u_s, yb_s, y_s, x1_s, h2_s, yp_s, kv_s = (scr[i * NS:(i + 1) * NS] for i in range(8))
    h_s, xn_s = (scr[8 * NS + 2 * i:8 * NS + 2 * i + 2] for i in range(2))

    sem_count = [0]
    dmas = {}

    def mk(name, src, dst):
        i = sem_count[0]
        sem_count[0] += 1
        cfg.setdefault("_sem_names", {})[i] = name
        dmas[name] = pltpu.make_async_copy(src, dst, sems.at[i])

    mk("c", c_hbm, c_s)
    mk("shift", shift_hbm, shift_s)
    mk("ssmd", ssmd_hbm, ssmd_s)
    for t in range(NS):
        r = pl.ds(t * TS, TS)
        for a in (2 * t, 2 * t + 1):
            mk(("ssmk", a), ssmk_hbm.at[:, pl.ds(a * C, C)], ssmk_s.bitcast(bf16).at[a])
        mk(("k", t), k_hbm.at[r, :], k_s.at[r, :])
        mk(("v", t), v_hbm.at[r, :], v_s.at[r, :])
        mk(("q", t), q_hbm.at[r, :], q_s.at[r, :])
        if t < NS - 1:
            mk(("out", t), out_s.at[r, :], o_hbm.at[r, :])
    r = pl.ds((NS - 1) * TS, TS)
    for j in range(NT):
        cs = pl.ds(j * LANES, LANES)
        mk(("outl", j), out_s.at[r, cs], o_hbm.at[r, cs])
    for j in range(6):
        cs = pl.ds(j * D, D)
        mk(("wmod", j), wmod_hbm.at[:, cs], wmod_s.at[:, cs])
    for j in range(F // LANES):
        cs = pl.ds(j * LANES, LANES)
        mk(("wg", j), wg_hbm.at[:, cs], wg_s.bitcast(bf16).at[j])
        mk(("wu", j), wu_hbm.at[:, cs], wu_s.bitcast(bf16).at[j])
    for j in range(NT):
        mk(("wd", j), wd_hbm.at[:, pl.ds(j * LANES, LANES)], wd_s.bitcast(bf16).at[j])

    order = ["c", "shift", "ssmd"]
    PP = NS
    pair = lambda t: [("ssmk", 2 * t), ("ssmk", 2 * t + 1), ("k", t), ("v", t)]
    for t in range(PP):
        order += pair(t)
    order += [("q", 0), ("q", 1)] + [("wmod", j) for j in range(5)]
    Q2 = cfg.get("q2_pos", 3)
    for j in range(F // LANES):
        order += [("wg", j), ("wu", j)]
        if j == Q2:
            order += [("q", 2)]
    order += [("wd", j) for j in range(NT)] + [("wmod", 5)]
    for t in range(PP, NS):
        order += pair(t)
        if t == PP:
            order += [("q", 3)]
    order += [("q", t) for t in range(3 if PP == NS else 4, NS)]
    for name in order:
        dmas[name].start()
    waited = set()

    def wait(*names):
        for n in names:
            if n not in waited:
                waited.add(n)
                if cfg.get("scopes", 0):
                    with jax.named_scope("w_" + (n if isinstance(n, str) else "%s%d" % n)):
                        dmas[n].wait()
                else:
                    dmas[n].wait()

    pk = lambda x: pltpu.bitcast(x.astype(bf16), jnp.uint32)
    upk = lambda x: pltpu.bitcast(x, bf16)

    def cat(vals):
        return vals[0] if len(vals) == 1 else jnp.concatenate(vals, axis=1)

    def table(f_off):
        f = lax.broadcasted_iota(jnp.int32, (C, C), 0)
        n = lax.broadcasted_iota(jnp.int32, (C, C), 1)
        m = ((4 * f + 1) * n + f_off) & (4 * C - 1)
        return jnp.sin(m.astype(f32) * (2.0 * math.pi / (4 * C)))

    t_cos, t_sin = table(C), table(0)

    wait("c", "shift", "ssmd")
    shift_rows = shift_s[...].astype(f32)
    ssmd = ssmd_s[...].astype(f32).reshape(1, D)
    cc = c_s[...].astype(f32)
    sc = jnp.broadcast_to((cc * jax.nn.sigmoid(cc)).astype(bf16), (16, D))
    never16 = jnp.abs(jnp.broadcast_to(cc[:, 0:LANES], (16, LANES))) < 0.0
    never = never16[0:8]
    zero = never16.astype(jnp.int32)[0, 0]
    zero2 = never16.astype(jnp.int32)[1, 1]
    f_s[zero] = pk(jnp.concatenate([t_cos, t_sin], axis=0))
    g_s[zero, 0] = pk(t_cos.T * (1.0 / C))
    g_s[zero, 1] = pk(t_sin.T * (1.0 / C))
    for j in range(4):
        tap_s[zero, j] = jnp.broadcast_to(shift_rows[j:j + 1, :], (8, D))
    sc_s[zero] = sc
    get_f = lambda: upk(f_s[zero2])
    get_g = lambda: jnp.concatenate([upk(g_s[zero2, 0]), upk(g_s[zero2, 1])], axis=1)

    queue = []
    state = {"last": None, "chain": [None, None]}

    def attach(results, budget):
        anchors = []
        for r in results:
            anchors += [(r, i, j) for j in range(r.shape[1] // LANES) for i in range(r.shape[0] // 16)]
        state["chain"] = [None, None]
        take, tot = [], 0
        while queue and tot < budget:
            take.append(queue.pop(0))
            tot += take[-1][1]
        pos = 0
        for fn, cost, _ in take:
            def get(frac=0.0, rows=8, pos=pos, cost=cost):
                r, i, j = anchors[min(int((pos + frac * cost) / max(tot, budget) * len(anchors)),
                                      len(anchors) - 1)]
                return r[i * 16:i * 16 + rows, j * LANES:(j + 1) * LANES]
            fn(get if cfg.get("anchor", 1) else None)
            pos += cost

    def flush(tag, extra=0):
        idx = [i for i, u in enumerate(queue) if u[2] == tag]
        if not idx:
            return
        n = idx[-1] + 1
        while extra > 0 and n < len(queue):
            extra -= queue[n][1]
            n += 1
        for fn, _, _ in queue[:n]:
            fn(None)
        del queue[:n]

    KR = 32

    def kvprep_units(t):
        r0 = t * TS
        units = []

        def head(jt, get):
            ls = slice(jt * LANES, (jt + 1) * LANES)
            if t == 0:
                kf_s[jt, 0:8, :] = jnp.zeros((8, LANES), f32)
            else:
                kf_s[jt, 0:8, :] = k_s[r0 - 16:r0, ls].astype(f32)[8:16]

        def unit(jt, g, get):
            ls = slice(jt * LANES, (jt + 1) * LANES)
            if g == 0:
                head(jt, get)
            rows = slice(r0 + g * KR, r0 + (g + 1) * KR)
            kb = k_s[rows, ls]
            vv = v_s[rows, ls].astype(f32)
            kk = kb.astype(f32)
            if get is not None:
                kk = jnp.concatenate([jnp.where(never16, get(0.0, 16), kk[0:16]), kk[16:]], axis=0)
            kf_s[jt, 8 + g * KR:8 + (g + 1) * KR, :] = kk
            wt = lambda j: jnp.concatenate([tap_s[zero2, j, :, ls]] * (KR // 8), axis=0)
            acc = kk * wt(0)
            for j in range(1, 4):
                acc = acc + kf_s[jt, 8 - j + g * KR:8 - j + (g + 1) * KR, :] * wt(j)
            kv_s[t][zero, jt, g * KR // 2:(g + 1) * KR // 2, :] = pk(acc * vv)

        for g in range(TS // KR):
            for jt in range(NT):
                units.append([functools.partial(unit, jt, g), 11 * KR // 8,
                              ("kv", 2 * t + g * KR // C)])
        return units

    def dft_k(a):
        t, o = a // 2, a % 2
        kc = upk(ssmk_s[a])
        kk = lax.dot_general(get_f(), kc, (((1,), (1,)), ((), ())), preferred_element_type=f32)
        kr, ki = kk[0:C], kk[C:2 * C]
        if a == 0:
            kr = kr + ssmd
        kp_s[t][zero, o, 0] = kr
        kp_s[t][zero, o, 1] = ki
        return kk

    def dft_u(a):
        t, o = a // 2, a % 2
        kv = cat([upk(kv_s[t][zero2, jt, o * C // 2:(o + 1) * C // 2, :]) for jt in range(NT)])
        uu = jnp.dot(get_f(), kv, preferred_element_type=f32)
        u_s[t][zero, o, 0] = uu[0:C]
        u_s[t][zero, o, 1] = uu[C:2 * C]
        return uu

    MG = cfg.get("mgrp", 4)

    def x_unit(t, jt, r, get):
        a0 = 2 * t
        ls = slice(jt * LANES, (jt + 1) * LANES)
        nm = a0 + 2
        res = []
        for hh in range(2):
            rs = slice(r * 16 + hh * 8, r * 16 + hh * 8 + 8)
            acc = [[None, None], [None, None]]
            us = None
            ldu = lambda n: (u_s[n // 2][zero2, n % 2, 0, rs, ls], u_s[n // 2][zero2, n % 2, 1, rs, ls])
            for m in range(nm):
                kr = kp_s[m // 2][zero2, m % 2, 0, rs, ls]
                ki = kp_s[m // 2][zero2, m % 2, 1, rs, ls]
                if m % MG == 0:
                    if get is not None:
                        an = get((hh * nm + m) / (2 * nm), 8)
                    else:
                        an = acc[0][0] if m else state["chain"][hh]
                    if an is not None:
                        kr = jnp.where(never, an, kr)
                        if get is None or cfg.get("anchor2", 0):
                            ki = jnp.where(never, an, ki)
                if m == 0:
                    us = [ldu(a0), ldu(a0 + 1)]
                else:
                    us = [ldu(a0 - m) if a0 - m >= 0 else None, us[0]]
                for o in range(2):
                    if us[o] is None:
                        continue
                    ur, ui = us[o]
                    pr = kr * ur - ki * ui
                    pi = kr * ui + ki * ur
                    acc[o][0] = pr if acc[o][0] is None else acc[o][0] + pr
                    acc[o][1] = pi if acc[o][1] is None else acc[o][1] + pi
            res.append(acc)
            state["chain"][hh] = acc[0][0]
        full = [[jnp.concatenate([res[0][o][p], res[1][o][p]], axis=0) for p in range(2)]
                for o in range(2)]
        rows = slice(r * 16, (r + 1) * 16)
        if t == 0:
            first = full[0]
        else:
            first = [full[0][0] + yp_s[t - 1][zero2, 1, rows, ls],
                     full[0][1] - yp_s[t - 1][zero2, 0, rows, ls]]
        second = [full[1][0] + full[0][1], full[1][1] - full[0][0]]
        if t + 1 < NS:
            yp_s[t][zero, 0, rows, ls] = full[1][0]
            yp_s[t][zero, 1, rows, ls] = full[1][1]
        for o, val in enumerate((first, second)):
            for p in range(2):
                yb_s[t][zero, o, jt, (p * C + r * 16) // 2:(p * C + (r + 1) * 16) // 2, :] = pk(val[p])

    def x_units(t):
        return [[functools.partial(x_unit, t, jt, r), 16 * (4 * t + 3) + 8, ("x", t)]
                for r in range(C // 16) for jt in range(NT)]

    def inv(t):
        res = []
        for o in range(2):
            yy = jnp.dot(get_g(), cat([upk(yb_s[t][zero2, o, jt]) for jt in range(NT)]),
                         preferred_element_type=f32)
            y_s[t][zero, o * C:(o + 1) * C, :] = yy
            res.append(yy)
        return res

    def modvec(j0, j1):
        wait(*[("wmod", j) for j in range(j0, j1)])
        m = jnp.dot(sc_s[zero2], wmod_s[:, j0 * D:j1 * D], preferred_element_type=f32)
        for j in range(j0, j1):
            mj = m[:, (j - j0) * D:(j - j0 + 1) * D]
            mod_s[zero, j] = mj + 1.0 if j in (1, 4) else mj
        return m

    def layernorm(x):
        mu = jnp.mean(x, axis=1, keepdims=True)
        xc = x - mu
        var = jnp.mean(xc * xc, axis=1, keepdims=True)
        return xc * lax.rsqrt(var + EPS)

    RG = 16
    mod = lambda j, cs=slice(None): mod_s[zero2, j, :, cs]

    def anchor_x(x, get):
        if get is None:
            return x
        return jnp.concatenate([jnp.where(never16, get(0.0, 16), x[:, 0:LANES]), x[:, LANES:]], axis=1)

    def put_h2(t, lr, val):
        for jt in range(NT):
            h2_s[t][zero, jt, lr.start // 2:lr.stop // 2, :] = pk(val[:, jt * LANES:(jt + 1) * LANES])

    def e1_unit(t, g, get):
        rows = slice(t * TS + g * RG, t * TS + (g + 1) * RG)
        lr = slice(g * RG, (g + 1) * RG)
        x = anchor_x(q_s[rows, :].astype(f32), get)
        h = layernorm(x) * mod(1) + mod(0)
        x1 = x + mod(2) * (h * y_s[t][zero2, lr, :])
        x1_s[t][zero, lr, :] = x1
        put_h2(t, lr, layernorm(x1) * mod(4) + mod(3))

    def e1ab_unit(t, g, get):
        rows = slice(t * TS + g * RG, t * TS + (g + 1) * RG)
        lr = slice(g * RG, (g + 1) * RG)
        x = anchor_x(q_s[rows, :].astype(f32), get)
        h = layernorm(x) * mod(1) + mod(0)
        x1 = x + mod(2) * (h * y_s[t][zero2, lr, :])
        x1_s[t][zero, lr, :] = x1
        xn_s[t][zero, lr, :] = layernorm(x1)

    def e1c_unit(t, g, get):
        lr = slice(g * RG, (g + 1) * RG)
        put_h2(t, lr, xn_s[t][zero2, lr, :] * mod(4) + mod(3))

    def units(fn, t, cost, tag):
        return [[functools.partial(fn, t, g), cost, (tag, t)] for g in range(TS // RG)]

    GB = cfg.get("glu_budget", 0.9)

    NTN = TN // LANES

    def glu_p1(t, j):
        tiles = range(j * NTN, (j + 1) * NTN)
        h2 = lambda: cat([upk(h2_s[t][zero2, jt]) for jt in range(NT)])
        g = jnp.dot(h2(), cat([upk(wg_s[w]) for w in tiles]), preferred_element_type=f32)
        u = jnp.dot(h2(), cat([upk(wu_s[w]) for w in tiles]), preferred_element_type=f32)
        hh = jnp.maximum(g, 0.0) * u
        for i, w in enumerate(tiles):
            h_s[t % 2][zero, w] = pk(hh[:, i * LANES:(i + 1) * LANES])
        attach([g, u], GB * 5 * TN)

    def glu_p2(t):
        for j in range(NT):
            wait(("wd", j))
        if t == 0:
            modvec(5, 6)
        for j in range(NT):
            cs = slice(j * LANES, (j + 1) * LANES)
            hh = cat([upk(h_s[t % 2][zero2, w]) for w in range(F // LANES)])
            d = jnp.dot(hh, upk(wd_s[j]), preferred_element_type=f32)
            gb = jnp.concatenate([mod(5, cs)] * (TS // 16), axis=0)
            out_s[t * TS:(t + 1) * TS, cs] = (x1_s[t][zero2, :, cs] + gb * d).astype(bf16)
            if t == NS - 1:
                dmas[("outl", j)].start()
            attach([d], GB * 768)
        if t < NS - 1:
            dmas[("out", t)].start()

    XP = cfg.get("xp", 4)
    PB = cfg.get("p1_budget", 4.5)
    MB = cfg.get("mod_budget", 3.0)
    FX = cfg.get("flush_extra", 0)
    state["inv"] = 0

    def do_inv(budget):
        t = state["inv"]
        flush(("x", t))
        attach(inv(t), budget)
        state["inv"] = t + 1

    for r in range(PP + 2):
        if r < PP:
            wait(("ssmk", 2 * r), ("ssmk", 2 * r + 1))
        if 1 <= r <= PP:
            wait(("k", r - 1), ("v", r - 1))
            queue[0:0] = kvprep_units(r - 1)
        for o in range(2):
            if r < PP:
                attach([dft_k(2 * r + o)], PB * 320)
            if r >= 2:
                flush(("kv", 2 * (r - 2) + 1))
                attach([dft_u(2 * (r - 2) + o)], PB * 320)
        if r >= 2:
            queue.extend(x_units(r - 2))

    MI = cfg.get("mod_inv", [2, 3, 4])

    def inv_upto(n):
        while state["inv"] < min(XP, n):
            do_inv(MB * 640)

    inv_upto(MI[0])
    attach([modvec(0, 3)], MB * 600)
    wait(("q", 0), ("q", 1))
    queue[0:0] = units(e1ab_unit, 0, 260, "e1ab") + units(e1ab_unit, 1, 260, "e1ab")
    inv_upto(MI[1])
    flush(("e1ab", 1), FX)
    inv_upto(MI[2])
    m34 = modvec(3, 5)
    queue[0:0] = units(e1c_unit, 0, 30, "e1c") + units(e1c_unit, 1, 30, "e1c")
    attach([m34], 32 * 30 - 1)
    flush(("e1c", 1))
    inv_upto(XP)

    def need_e1(t):
        wait(*[("q", tt) for tt in range(t, NS if t > 2 else t + 1)])
        while state["inv"] <= t:
            do_inv(GB * 640)
        rest = list(queue)
        del queue[:]
        for un in units(e1_unit, t, 300, "e1"):
            queue.append(un)
            gap = cfg.get("e1_gap", 0)
            while gap > 0:
                queue.append(rest.pop(0) if rest else [lambda get: None, gap, None])
                gap -= queue[-1][1]
        queue.extend(rest)

    j0 = 0
    e2_done = False
    for gr in cfg.get("groups", [1, 2, 3, 3, 3]):
        js = range(j0, min(j0 + gr, NF))
        j0 += gr
        for j in js:
            for w in range(j * NTN, (j + 1) * NTN):
                wait(("wg", w), ("wu", w))
        if j0 - gr >= cfg.get("e2_at", 6) and not e2_done:
            need_e1(2)
            e2_done = True
        for t in range(2):
            for j in js:
                glu_p1(t, j)
    assert j0 >= NF and e2_done
    LA = cfg.get("lookahead", 2)
    EARLY = cfg.get("e1_early", 1)
    glu_p2(0)
    for t in range(1, NS):
        if t + 1 < NS:
            flush(("e1", t + 1))
        if EARLY and t + 2 < NS:
            need_e1(t + 2)
        if t + 1 < NS:
            for j in range(LA):
                glu_p1(t + 1, j)
        glu_p2(t)
        if not EARLY and t + 2 < NS:
            need_e1(t + 2)
        if t + 1 < NS:
            for j in range(LA, NF):
                glu_p1(t + 1, j)
    assert len(waited) == len(order)
    if cfg.get("scopes", 0):
        with jax.named_scope("w_end0"):
            dmas[("out", 0)].wait()
        dmas[("out", 0)].start()
    for t in range(NS - 1):
        dmas[("out", t)].wait()
    for j in range(NT):
        dmas[("outl", j)].wait()


def _build(S, D, F, cfg):
    f32, bf16, u32 = jnp.float32, jnp.bfloat16, jnp.uint32
    NT, NA, TS, NS = D // LANES, S // C, 2 * C, S // (2 * C)
    scratch = [
        pltpu.VMEM((S, D), bf16),
        pltpu.VMEM((S, D), bf16),
        pltpu.VMEM((S, D), bf16),
        pltpu.VMEM((NA, D // 2, LANES), u32),
        pltpu.VMEM((F // LANES, D // 2, LANES), u32),
        pltpu.VMEM((F // LANES, D // 2, LANES), u32),
        pltpu.VMEM((NT, F // 2, LANES), u32),
        pltpu.VMEM((D, 6 * D), bf16),
        pltpu.VMEM((4, D), bf16),
        pltpu.VMEM((D,), bf16),
        pltpu.VMEM((1, D), bf16),
        pltpu.VMEM((NT, 8 + TS, LANES), f32),
        pltpu.VMEM((S, D), bf16),
        pltpu.SemaphoreType.DMA((112,)),
        pltpu.VMEM((1, C, C), u32),
        pltpu.VMEM((1, 2, C // 2, C), u32),
        pltpu.VMEM((1, 4, 8, D), f32),
        pltpu.VMEM((1, 16, D), bf16),
        pltpu.VMEM((1, 6, 16, D), f32),
    ]
    scratch += [pltpu.VMEM((1, 2, 2, C, D), f32) for _ in range(NS)]
    scratch += [pltpu.VMEM((1, 2, 2, C, D), f32) for _ in range(NS)]
    scratch += [pltpu.VMEM((1, 2, NT, C, LANES), u32) for _ in range(NS)]
    scratch += [pltpu.VMEM((1, TS, D), f32) for _ in range(NS)]
    scratch += [pltpu.VMEM((1, TS, D), f32) for _ in range(NS)]
    scratch += [pltpu.VMEM((1, NT, TS // 2, LANES), u32) for _ in range(NS)]
    scratch += [pltpu.VMEM((1, 2, C, D), f32) for _ in range(NS)]
    scratch += [pltpu.VMEM((1, NT, TS // 2, LANES), u32) for _ in range(NS)]
    scratch += [pltpu.VMEM((1, F // LANES, TS // 2, LANES), u32) for _ in range(2)]
    scratch += [pltpu.VMEM((1, TS, D), f32) for _ in range(2)]
    return pl.pallas_call(
        functools.partial(_kernel, S=S, D=D, F=F, cfg=cfg),
        in_specs=[pl.BlockSpec(memory_space=pl.ANY)] * 11,
        out_specs=pl.BlockSpec(memory_space=pl.ANY),
        out_shape=jax.ShapeDtypeStruct((S, D), bf16),
        scratch_shapes=scratch,
        compiler_params=pltpu.CompilerParams(vmem_limit_bytes=112 * 1024 * 1024),
    )


def _run(A_q, A_k, A_v, A_shift_k, A_ssm_k, A_ssm_D, B_x, B_W_gate, B_W_up, B_W_down, c, w_mod,
         cfg):
    del B_x
    B, S, D = A_q.shape
    F = B_W_gate.shape[1]
    assert B == 1
    assert A_shift_k.shape[1] == 4
    out = _build(S, D, F, cfg)(
        A_q.reshape(S, D), A_k.reshape(S, D), A_v.reshape(S, D), A_shift_k.T, A_ssm_k,
        A_ssm_D, B_W_gate, B_W_up, B_W_down, c, w_mod)
    return out.reshape(B, S, D)


@jax.jit
def pallas_adaLN_cond__ssm_conv_h3__glu_gated_reglu__prompt_kernel(
    A_q: jax.Array,
    A_k: jax.Array,
    A_v: jax.Array,
    A_shift_k: jax.Array,
    A_ssm_k: jax.Array,
    A_ssm_D: jax.Array,
    B_x: jax.Array,
    B_W_gate: jax.Array,
    B_W_up: jax.Array,
    B_W_down: jax.Array,
    c: jax.Array,
    w_mod: jax.Array,
):
    return _run(A_q, A_k, A_v, A_shift_k, A_ssm_k, A_ssm_D, B_x, B_W_gate, B_W_up, B_W_down,
                c, w_mod, {})
```

```python
import functools
import math

import jax
import jax.numpy as jnp
import numpy as np
from jax import lax
import jax.experimental.pallas as pl
import jax.experimental.pallas.tpu as pltpu

C = 128
LANES = 128
EPS = 1e-5


def _kernel(q_hbm, k_hbm, v_hbm, shift_hbm, ssmk_hbm, ssmd_hbm, wg_hbm, wu_hbm, wd_hbm,
            c_hbm, wmod_hbm, o_hbm, *scr, S, D, F, cfg):
    f32, bf16 = jnp.float32, jnp.bfloat16
    NT = D // LANES
    TS = 2 * C
    NS = S // TS
    TN = cfg.get("tn", 128)
    NF = F // TN
    (q_s, k_s, v_s, ssmk_s, wg_s, wu_s, wd_s, wmod_s, shift_s, ssmd_s, c_s,
     kf_s, out_s, sems, f_s, g_s, tap_s, sc_s, mod_s) = scr[:19]
    scr = scr[19:]
    kp_s, u_s, yb_s, y_s, x1_s, h2_s, yp_s, kv_s = (scr[i * NS:(i + 1) * NS] for i in range(8))
    h_s, xn_s = (scr[8 * NS + 2 * i:8 * NS + 2 * i + 2] for i in range(2))

    sem_count = [0]
    dmas = {}

    def mk(name, src, dst):
        i = sem_count[0]
        sem_count[0] += 1
        dmas[name] = pltpu.make_async_copy(src, dst, sems.at[i])

    mk("c", c_hbm, c_s)
    mk("shift", shift_hbm, shift_s)
    mk("ssmd", ssmd_hbm, ssmd_s)
    for t in range(NS):
        r = pl.ds(t * TS, TS)
        for a in (2 * t, 2 * t + 1):
            mk(("ssmk", a), ssmk_hbm.at[:, pl.ds(a * C, C)], ssmk_s.bitcast(bf16).at[a])
        mk(("k", t), k_hbm.at[r, :], k_s.at[r, :])
        mk(("v", t), v_hbm.at[r, :], v_s.at[r, :])
        mk(("q", t), q_hbm.at[r, :], q_s.at[r, :])
        if t < NS - 1:
            mk(("out", t), out_s.at[r, :], o_hbm.at[r, :])
    r = pl.ds((NS - 1) * TS, TS)
    for j in range(NT):
        cs = pl.ds(j * LANES, LANES)
        mk(("outl", j), out_s.at[r, cs], o_hbm.at[r, cs])
    for j in range(6):
        cs = pl.ds(j * D, D)
        mk(("wmod", j), wmod_hbm.at[:, cs], wmod_s.at[:, cs])
    for j in range(F // LANES):
        cs = pl.ds(j * LANES, LANES)
        mk(("wg", j), wg_hbm.at[:, cs], wg_s.bitcast(bf16).at[j])
        mk(("wu", j), wu_hbm.at[:, cs], wu_s.bitcast(bf16).at[j])
    for j in range(NT):
        mk(("wd", j), wd_hbm.at[:, pl.ds(j * LANES, LANES)], wd_s.bitcast(bf16).at[j])

    order = ["c", "shift", "ssmd"]
    pair = lambda t: [("ssmk", 2 * t), ("ssmk", 2 * t + 1), ("k", t), ("v", t)]
    for t in range(NS):
        order += pair(t)
    order += [("q", 0), ("q", 1)] + [("wmod", j) for j in range(5)]
    Q2 = cfg.get("q2_pos", 11)
    for j in range(F // LANES):
        order += [("wg", j), ("wu", j)]
        if j == Q2:
            order += [("q", 2)]
    order += [("wd", j) for j in range(NT)] + [("wmod", 5)]
    order += [("q", t) for t in range(3, NS)]
    for name in order:
        dmas[name].start()
    waited = set()

    def wait(*names):
        for n in names:
            if n not in waited:
                waited.add(n)
                dmas[n].wait()

    pk = lambda x: pltpu.bitcast(x.astype(bf16), jnp.uint32)
    upk = lambda x: pltpu.bitcast(x, bf16)

    def cat(vals):
        return vals[0] if len(vals) == 1 else jnp.concatenate(vals, axis=1)

    def table(f_off):
        f = lax.broadcasted_iota(jnp.int32, (C, C), 0)
        n = lax.broadcasted_iota(jnp.int32, (C, C), 1)
        m = ((4 * f + 1) * n + f_off) & (4 * C - 1)
        return jnp.sin(m.astype(f32) * (2.0 * math.pi / (4 * C)))

    t_cos, t_sin = table(C), table(0)

    wait("c", "shift", "ssmd")
    shift_rows = shift_s[...].astype(f32)
    ssmd = ssmd_s[...].astype(f32).reshape(1, D)
    cc = c_s[...].astype(f32)
    sc = jnp.broadcast_to((cc * jax.nn.sigmoid(cc)).astype(bf16), (16, D))
    never16 = jnp.abs(jnp.broadcast_to(cc[:, 0:LANES], (16, LANES))) < 0.0
    never = never16[0:8]
    zero = never16.astype(jnp.int32)[0, 0]
    zero2 = never16.astype(jnp.int32)[1, 1]
    f_s[zero] = pk(jnp.concatenate([t_cos, t_sin], axis=0))
    g_s[zero, 0] = pk(t_cos.T * (1.0 / C))
    g_s[zero, 1] = pk(t_sin.T * (1.0 / C))
    for j in range(4):
        tap_s[zero, j] = jnp.broadcast_to(shift_rows[j:j + 1, :], (8, D))
    sc_s[zero] = sc
    get_f = lambda: upk(f_s[zero2])
    get_g = lambda: jnp.concatenate([upk(g_s[zero2, 0]), upk(g_s[zero2, 1])], axis=1)

    queue = []
    state = {"chain": [None, None]}

    def attach(results, budget):
        anchors = []
        for r in results:
            anchors += [(r, i, j) for j in range(r.shape[1] // LANES) for i in range(r.shape[0] // 16)]
        state["chain"] = [None, None]
        take, tot = [], 0
        while queue and tot < budget:
            take.append(queue.pop(0))
            tot += take[-1][1]
        pos = 0
        for fn, cost, _ in take:
            def get(frac=0.0, rows=8, pos=pos, cost=cost):
                r, i, j = anchors[min(int((pos + frac * cost) / max(tot, budget) * len(anchors)),
                                      len(anchors) - 1)]
                return r[i * 16:i * 16 + rows, j * LANES:(j + 1) * LANES]
            fn(get)
            pos += cost

    def flush(tag):
        idx = [i for i, u in enumerate(queue) if u[2] == tag]
        n = idx[-1] + 1 if idx else 0
        for fn, _, _ in queue[:n]:
            fn(None)
        del queue[:n]

    KR = 32

    def kvprep_units(t):
        r0 = t * TS
        units = []

        def head(jt, get):
            ls = slice(jt * LANES, (jt + 1) * LANES)
            if t == 0:
                kf_s[jt, 0:8, :] = jnp.zeros((8, LANES), f32)
            else:
                kf_s[jt, 0:8, :] = k_s[r0 - 16:r0, ls].astype(f32)[8:16]

        def unit(jt, g, get):
            ls = slice(jt * LANES, (jt + 1) * LANES)
            if g == 0:
                head(jt, get)
            rows = slice(r0 + g * KR, r0 + (g + 1) * KR)
            kb = k_s[rows, ls]
            vv = v_s[rows, ls].astype(f32)
            kk = kb.astype(f32)
            if get is not None:
                kk = jnp.concatenate([jnp.where(never16, get(0.0, 16), kk[0:16]), kk[16:]], axis=0)
            kf_s[jt, 8 + g * KR:8 + (g + 1) * KR, :] = kk
            wt = lambda j: jnp.concatenate([tap_s[zero2, j, :, ls]] * (KR // 8), axis=0)
            acc = kk * wt(0)
            for j in range(1, 4):
                acc = acc + kf_s[jt, 8 - j + g * KR:8 - j + (g + 1) * KR, :] * wt(j)
            kv_s[t][zero, jt, g * KR // 2:(g + 1) * KR // 2, :] = pk(acc * vv)

        for g in range(TS // KR):
            for jt in range(NT):
                units.append([functools.partial(unit, jt, g), 11 * KR // 8,
                              ("kv", 2 * t + g * KR // C)])
        return units

    def dft_k(a):
        t, o = a // 2, a % 2
        kc = upk(ssmk_s[a])
        kk = lax.dot_general(get_f(), kc, (((1,), (1,)), ((), ())), preferred_element_type=f32)
        kr, ki = kk[0:C], kk[C:2 * C]
        if a == 0:
            kr = kr + ssmd
        kp_s[t][zero, o, 0] = kr
        kp_s[t][zero, o, 1] = ki
        return kk

    def dft_u(a):
        t, o = a // 2, a % 2
        kv = cat([upk(kv_s[t][zero2, jt, o * C // 2:(o + 1) * C // 2, :]) for jt in range(NT)])
        uu = jnp.dot(get_f(), kv, preferred_element_type=f32)
        u_s[t][zero, o, 0] = uu[0:C]
        u_s[t][zero, o, 1] = uu[C:2 * C]
        return uu

    MG = cfg.get("mgrp", 4)

    def x_unit(t, jt, r, get):
        a0 = 2 * t
        ls = slice(jt * LANES, (jt + 1) * LANES)
        nm = a0 + 2
        res = []
        for hh in range(2):
            rs = slice(r * 16 + hh * 8, r * 16 + hh * 8 + 8)
            acc = [[None, None], [None, None]]
            us = None
            ldu = lambda n: (u_s[n // 2][zero2, n % 2, 0, rs, ls], u_s[n // 2][zero2, n % 2, 1, rs, ls])
            for m in range(nm):
                kr = kp_s[m // 2][zero2, m % 2, 0, rs, ls]
                ki = kp_s[m // 2][zero2, m % 2, 1, rs, ls]
                if m % MG == 0:
                    if get is not None:
                        an = get((hh * nm + m) / (2 * nm), 8)
                    else:
                        an = acc[0][0] if m else state["chain"][hh]
                    if an is not None:
                        kr = jnp.where(never, an, kr)
                        if get is None:
                            ki = jnp.where(never, an, ki)
                if m == 0:
                    us = [ldu(a0), ldu(a0 + 1)]
                else:
                    us = [ldu(a0 - m) if a0 - m >= 0 else None, us[0]]
                for o in range(2):
                    if us[o] is None:
                        continue
                    ur, ui = us[o]
                    pr = kr * ur - ki * ui
                    pi = kr * ui + ki * ur
                    acc[o][0] = pr if acc[o][0] is None else acc[o][0] + pr
                    acc[o][1] = pi if acc[o][1] is None else acc[o][1] + pi
            res.append(acc)
            state["chain"][hh] = acc[0][0]
        full = [[jnp.concatenate([res[0][o][p], res[1][o][p]], axis=0) for p in range(2)]
                for o in range(2)]
        rows = slice(r * 16, (r + 1) * 16)
        if t == 0:
            first = full[0]
        else:
            first = [full[0][0] + yp_s[t - 1][zero2, 1, rows, ls],
                     full[0][1] - yp_s[t - 1][zero2, 0, rows, ls]]
        second = [full[1][0] + full[0][1], full[1][1] - full[0][0]]
        if t + 1 < NS:
            yp_s[t][zero, 0, rows, ls] = full[1][0]
            yp_s[t][zero, 1, rows, ls] = full[1][1]
        for o, val in enumerate((first, second)):
            for p in range(2):
                yb_s[t][zero, o, jt, (p * C + r * 16) // 2:(p * C + (r + 1) * 16) // 2, :] = pk(val[p])

    def x_units(t):
        return [[functools.partial(x_unit, t, jt, r), 16 * (4 * t + 3) + 8, ("x", t)]
                for r in range(C // 16) for jt in range(NT)]

    def inv(t):
        res = []
        for o in range(2):
            yy = jnp.dot(get_g(), cat([upk(yb_s[t][zero2, o, jt]) for jt in range(NT)]),
                         preferred_element_type=f32)
            y_s[t][zero, o * C:(o + 1) * C, :] = yy
            res.append(yy)
        return res

    def modvec(j0, j1):
        wait(*[("wmod", j) for j in range(j0, j1)])
        m = jnp.dot(sc_s[zero2], wmod_s[:, j0 * D:j1 * D], preferred_element_type=f32)
        for j in range(j0, j1):
            mj = m[:, (j - j0) * D:(j - j0 + 1) * D]
            mod_s[zero, j] = mj + 1.0 if j in (1, 4) else mj
        return m

    def layernorm(x):
        mu = jnp.mean(x, axis=1, keepdims=True)
        xc = x - mu
        var = jnp.mean(xc * xc, axis=1, keepdims=True)
        return xc * lax.rsqrt(var + EPS)

    RG = 16
    mod = lambda j, cs=slice(None): mod_s[zero2, j, :, cs]

    def anchor_x(x, get):
        if get is None:
            return x
        return jnp.concatenate([jnp.where(never16, get(0.0, 16), x[:, 0:LANES]), x[:, LANES:]], axis=1)

    def put_h2(t, lr, val):
        for jt in range(NT):
            h2_s[t][zero, jt, lr.start // 2:lr.stop // 2, :] = pk(val[:, jt * LANES:(jt + 1) * LANES])

    def e1_unit(t, g, get):
        rows = slice(t * TS + g * RG, t * TS + (g + 1) * RG)
        lr = slice(g * RG, (g + 1) * RG)
        x = anchor_x(q_s[rows, :].astype(f32), get)
        h = layernorm(x) * mod(1) + mod(0)
        x1 = x + mod(2) * (h * y_s[t][zero2, lr, :])
        x1_s[t][zero, lr, :] = x1
        put_h2(t, lr, layernorm(x1) * mod(4) + mod(3))

    def e1ab_unit(t, g, get):
        rows = slice(t * TS + g * RG, t * TS + (g + 1) * RG)
        lr = slice(g * RG, (g + 1) * RG)
        x = anchor_x(q_s[rows, :].astype(f32), get)
        h = layernorm(x) * mod(1) + mod(0)
        x1 = x + mod(2) * (h * y_s[t][zero2, lr, :])
        x1_s[t][zero, lr, :] = x1
        xn_s[t][zero, lr, :] = layernorm(x1)

    def e1c_unit(t, g, get):
        lr = slice(g * RG, (g + 1) * RG)
        put_h2(t, lr, xn_s[t][zero2, lr, :] * mod(4) + mod(3))

    def units(fn, t, cost, tag):
        return [[functools.partial(fn, t, g), cost, (tag, t)] for g in range(TS // RG)]

    GB = cfg.get("glu_budget", 0.9)

    NTN = TN // LANES

    def glu_p1(t, j):
        tiles = range(j * NTN, (j + 1) * NTN)
        h2 = lambda: cat([upk(h2_s[t][zero2, jt]) for jt in range(NT)])
        g = jnp.dot(h2(), cat([upk(wg_s[w]) for w in tiles]), preferred_element_type=f32)
        u = jnp.dot(h2(), cat([upk(wu_s[w]) for w in tiles]), preferred_element_type=f32)
        hh = jnp.maximum(g, 0.0) * u
        for i, w in enumerate(tiles):
            h_s[t % 2][zero, w] = pk(hh[:, i * LANES:(i + 1) * LANES])
        attach([g, u], GB * 5 * TN)

    def glu_p2(t):
        for j in range(NT):
            wait(("wd", j))
        if t == 0:
            modvec(5, 6)
        for j in range(NT):
            cs = slice(j * LANES, (j + 1) * LANES)
            hh = cat([upk(h_s[t % 2][zero2, w]) for w in range(F // LANES)])
            d = jnp.dot(hh, upk(wd_s[j]), preferred_element_type=f32)
            gb = jnp.concatenate([mod(5, cs)] * (TS // 16), axis=0)
            out_s[t * TS:(t + 1) * TS, cs] = (x1_s[t][zero2, :, cs] + gb * d).astype(bf16)
            if t == NS - 1:
                dmas[("outl", j)].start()
            attach([d], GB * 768)
        if t < NS - 1:
            dmas[("out", t)].start()

    XP = cfg.get("xp", 4)
    PB = cfg.get("p1_budget", 4.5)
    MB = cfg.get("mod_budget", 3.0)
    state["inv"] = 0

    def do_inv(budget):
        t = state["inv"]
        flush(("x", t))
        attach(inv(t), budget)
        state["inv"] = t + 1

    for r in range(NS + 2):
        if r < NS:
            wait(("ssmk", 2 * r), ("ssmk", 2 * r + 1))
        if 1 <= r <= NS:
            wait(("k", r - 1), ("v", r - 1))
            queue[0:0] = kvprep_units(r - 1)
        for o in range(2):
            if r < NS:
                attach([dft_k(2 * r + o)], PB * 320)
            if r >= 2:
                flush(("kv", 2 * (r - 2) + 1))
                attach([dft_u(2 * (r - 2) + o)], PB * 320)
        if r >= 2:
            queue.extend(x_units(r - 2))

    MI = cfg.get("mod_inv", [3, 4, 4])

    def inv_upto(n):
        while state["inv"] < min(XP, n):
            do_inv(MB * 640)

    inv_upto(MI[0])
    attach([modvec(0, 3)], MB * 600)
    wait(("q", 0), ("q", 1))
    queue[0:0] = units(e1ab_unit, 0, 260, "e1ab") + units(e1ab_unit, 1, 260, "e1ab")
    inv_upto(MI[1])
    flush(("e1ab", 1))
    inv_upto(MI[2])
    m34 = modvec(3, 5)
    queue[0:0] = units(e1c_unit, 0, 30, "e1c") + units(e1c_unit, 1, 30, "e1c")
    attach([m34], 32 * 30 - 1)
    flush(("e1c", 1))
    inv_upto(XP)

    def need_e1(t):
        wait(*[("q", tt) for tt in range(t, NS if t > 2 else t + 1)])
        while state["inv"] <= t:
            do_inv(GB * 640)
        queue[0:0] = units(e1_unit, t, 300, "e1")

    j0 = 0
    e2_done = False
    for gr in cfg.get("groups", [1, 3, 4, 4]):
        js = range(j0, min(j0 + gr, NF))
        j0 += gr
        for j in js:
            for w in range(j * NTN, (j + 1) * NTN):
                wait(("wg", w), ("wu", w))
        if j0 - gr >= cfg.get("e2_at", 8) and not e2_done:
            need_e1(2)
            e2_done = True
        for t in range(2):
            for j in js:
                glu_p1(t, j)
    assert j0 >= NF and e2_done
    LA = cfg.get("lookahead", 2)
    glu_p2(0)
    for t in range(1, NS):
        if t + 1 < NS:
            flush(("e1", t + 1))
        if t + 2 < NS:
            need_e1(t + 2)
        if t + 1 < NS:
            for j in range(LA):
                glu_p1(t + 1, j)
        glu_p2(t)
        if t + 1 < NS:
            for j in range(LA, NF):
                glu_p1(t + 1, j)
    assert len(waited) == len(order)
    for t in range(NS - 1):
        dmas[("out", t)].wait()
    for j in range(NT):
        dmas[("outl", j)].wait()


def _build(S, D, F, cfg):
    f32, bf16, u32 = jnp.float32, jnp.bfloat16, jnp.uint32
    NT, NA, TS, NS = D // LANES, S // C, 2 * C, S // (2 * C)
    scratch = [
        pltpu.VMEM((S, D), bf16),
        pltpu.VMEM((S, D), bf16),
        pltpu.VMEM((S, D), bf16),
        pltpu.VMEM((NA, D // 2, LANES), u32),
        pltpu.VMEM((F // LANES, D // 2, LANES), u32),
        pltpu.VMEM((F // LANES, D // 2, LANES), u32),
        pltpu.VMEM((NT, F // 2, LANES), u32),
        pltpu.VMEM((D, 6 * D), bf16),
        pltpu.VMEM((4, D), bf16),
        pltpu.VMEM((D,), bf16),
        pltpu.VMEM((1, D), bf16),
        pltpu.VMEM((NT, 8 + TS, LANES), f32),
        pltpu.VMEM((S, D), bf16),
        pltpu.SemaphoreType.DMA((112,)),
        pltpu.VMEM((1, C, C), u32),
        pltpu.VMEM((1, 2, C // 2, C), u32),
        pltpu.VMEM((1, 4, 8, D), f32),
        pltpu.VMEM((1, 16, D), bf16),
        pltpu.VMEM((1, 6, 16, D), f32),
    ]
    scratch += [pltpu.VMEM((1, 2, 2, C, D), f32) for _ in range(NS)]
    scratch += [pltpu.VMEM((1, 2, 2, C, D), f32) for _ in range(NS)]
    scratch += [pltpu.VMEM((1, 2, NT, C, LANES), u32) for _ in range(NS)]
    scratch += [pltpu.VMEM((1, TS, D), f32) for _ in range(NS)]
    scratch += [pltpu.VMEM((1, TS, D), f32) for _ in range(NS)]
    scratch += [pltpu.VMEM((1, NT, TS // 2, LANES), u32) for _ in range(NS)]
    scratch += [pltpu.VMEM((1, 2, C, D), f32) for _ in range(NS)]
    scratch += [pltpu.VMEM((1, NT, TS // 2, LANES), u32) for _ in range(NS)]
    scratch += [pltpu.VMEM((1, F // LANES, TS // 2, LANES), u32) for _ in range(2)]
    scratch += [pltpu.VMEM((1, TS, D), f32) for _ in range(2)]
    return pl.pallas_call(
        functools.partial(_kernel, S=S, D=D, F=F, cfg=cfg),
        in_specs=[pl.BlockSpec(memory_space=pl.ANY)] * 11,
        out_specs=pl.BlockSpec(memory_space=pl.ANY),
        out_shape=jax.ShapeDtypeStruct((S, D), bf16),
        scratch_shapes=scratch,
        compiler_params=pltpu.CompilerParams(vmem_limit_bytes=112 * 1024 * 1024),
    )


def _run(A_q, A_k, A_v, A_shift_k, A_ssm_k, A_ssm_D, B_x, B_W_gate, B_W_up, B_W_down, c, w_mod,
         cfg):
    del B_x
    B, S, D = A_q.shape
    F = B_W_gate.shape[1]
    assert B == 1
    assert A_shift_k.shape[1] == 4
    out = _build(S, D, F, cfg)(
        A_q.reshape(S, D), A_k.reshape(S, D), A_v.reshape(S, D), A_shift_k.T, A_ssm_k,
        A_ssm_D, B_W_gate, B_W_up, B_W_down, c, w_mod)
    return out.reshape(B, S, D)


@jax.jit
def pallas_adaLN_cond__ssm_conv_h3__glu_gated_reglu__prompt_kernel(
    A_q: jax.Array,
    A_k: jax.Array,
    A_v: jax.Array,
    A_shift_k: jax.Array,
    A_ssm_k: jax.Array,
    A_ssm_D: jax.Array,
    B_x: jax.Array,
    B_W_gate: jax.Array,
    B_W_up: jax.Array,
    B_W_down: jax.Array,
    c: jax.Array,
    w_mod: jax.Array,
):
    return _run(A_q, A_k, A_v, A_shift_k, A_ssm_k, A_ssm_D, B_x, B_W_gate, B_W_up, B_W_down,
                c, w_mod, {})
```
